```python
import os as _os
_os.environ.setdefault("JAX_PLATFORMS", "cpu")
import jax
import jax.numpy as jnp

def _softmax(x, axis=-1):
    return jax.nn.softmax(x, axis=axis)
def _gelu(x):
    return jax.nn.gelu(x, approximate=True)
def _silu(x):
    return jax.nn.silu(x)
def _sigmoid(x):
    return jax.nn.sigmoid(x)
def _layernorm(x, axis=-1, eps=1e-5):
    m = jnp.mean(x, axis=axis, keepdims=True)
    v = jnp.var(x, axis=axis, keepdims=True)
    return (x - m) / jnp.sqrt(v + eps)
def _scatter_add(tgt, idx, src, axis=0):
    return tgt.at[idx].add(src)
def _segment_sum(src, seg, n):
    return jax.ops.segment_sum(src, seg, n)
class _Rng:
    def __init__(self, key):
        self._k = key
    def _next(self):
        self._k, sub = jax.random.split(self._k)
        return sub
    def normal(self, shape):
        return jax.random.normal(self._next(), shape, dtype=jnp.bfloat16)
    def randint(self, lo, hi, shape):
        return jax.random.randint(self._next(), shape, lo, hi, dtype=jnp.int32)
    def uniform(self, shape, lo=0.0, hi=1.0):
        return jax.random.uniform(self._next(), shape, jnp.bfloat16, lo, hi)
    def permutation(self, n):
        return jax.random.permutation(self._next(), n)


kernel_name = 'interleave_layers__ssm_conv_h3__dense_activation_silu__prompt'

def setup_inputs():
    _rng = _Rng(jax.random.key(int.from_bytes(__import__("os").urandom(4), "little")))
    _w = (lambda a: (lambda t: t.astype(jnp.bfloat16) if jnp.issubdtype(t.dtype, jnp.floating) else t)(jnp.asarray(a)))
    def _A_setup():
        B, S, D = 1, 2048, 448
        ks = 4
        return {
            "q": _w((lambda *s: _rng.normal(s) * 0.05)(B, S, D)),
            "k": _w((lambda *s: _rng.normal(s) * 0.2)(B, S, D)),
            "v": _w((lambda *s: _rng.normal(s) * 0.2)(B, S, D)),
            "shift_k": _w((lambda *s: _rng.normal(s) * 0.2)(D, ks) * 0.5),
            "ssm_k": _w((lambda *s: _rng.normal(s) * 0.2)(D, S) * (1.0 / S ** 0.5)),
            "ssm_D": _w((lambda *s: _rng.normal(s) * 0.2)(D)),
        }
    _A_in = _A_setup()

    def _B_setup():
        B, S, D, F = 1, 2048, 448, 1792
        return {
            "x": _w((lambda *s: _rng.normal(s) * 0.05)(B, S, D)),
            "w1": _w((lambda *s: _rng.normal(s) * 0.2)(D, F) * (D ** -0.5)),
            "w2": _w((lambda *s: _rng.normal(s) * 0.2)(F, D) * (F ** -0.5)),
        }
    _B_in = _B_setup()

    return {
        "A_q": _A_in["q"],
        "A_k": _A_in["k"],
        "A_v": _A_in["v"],
        "A_shift_k": _A_in["shift_k"],
        "A_ssm_k": _A_in["ssm_k"],
        "A_ssm_D": _A_in["ssm_D"],
        "B_x": _B_in["x"],
        "B_w1": _B_in["w1"],
        "B_w2": _B_in["w2"],
    }

def reference(A_q, A_k, A_v, A_shift_k, A_ssm_k, A_ssm_D, B_x, B_w1, B_w2):
    def _A_ref(q, k, v, shift_k, ssm_k, ssm_D):
        B, S, D = q.shape
        ks = shift_k.shape[-1]
        k_pad = jnp.pad(k, ((0, 0), (ks - 1, 0), (0, 0)))
        k_shift = jnp.zeros_like(k)
        for t in range(ks):
            k_shift = k_shift + k_pad[:, t:t + S, :] * shift_k[:, ks - 1 - t][None, None, :]
        kv = k_shift * v
        L = 2 * S
        kv_pad = jnp.pad(kv, ((0, 0), (0, S), (0, 0)))
        kf_pad = jnp.pad(ssm_k, ((0, 0), (0, S)))
        kv_f = (lambda x, axes=(-2,-1): jnp.fft.rfft2(x.astype(jnp.float32), axes=axes))(kv_pad[:, None, :, :], axes=(1, 2))
        kf_f = (lambda x, axes=(-2,-1): jnp.fft.rfft2(x.astype(jnp.float32), axes=axes))(kf_pad[:, None, :], axes=(1, 2))
        kf_f = (lambda x, *d: x.transpose(*d))(kf_f, 1, 2, 0)
        y_f = kv_f * kf_f[None, :, :, :]
        y = (lambda x, s, axes=(-2,-1): jnp.fft.irfft2(x, s=s, axes=axes).astype(jnp.bfloat16))(y_f, (1, L), axes=(1, 2))[:, 0, :S, :]
        y = y + kv * ssm_D[None, None, :]
        return q * y

    def _B_ref(x, w1, w2):
        h = jnp.einsum("bsd,df->bsf", x, w1)
        h = _silu(h)
        out = jnp.einsum("bsf,fd->bsd", h, w2)
        return out

    x = A_q
    x = x + _A_ref(_layernorm(x, axis=-1), A_k, A_v, A_shift_k, A_ssm_k, A_ssm_D)
    x = x + _B_ref(_layernorm(x, axis=-1), B_w1, B_w2)
    x = x + _A_ref(_layernorm(x, axis=-1), A_k, A_v, A_shift_k, A_ssm_k, A_ssm_D)
    x = x + _B_ref(_layernorm(x, axis=-1), B_w1, B_w2)
    return x
```

```python
import jax
import jax.numpy as jnp
import numpy as np
from jax import lax
import jax.experimental.pallas as pl
import jax.experimental.pallas.tpu as pltpu

S, D, F = 2048, 448, 1792
BK = 128
NB = S // BK
T = 512
Q = T // BK
NS = S // T
W1C = 2
RG = 112
NG = D // RG
PG = RG // 8
RC = 16
EPS = 1e-5
f32, bf16, u32 = jnp.float32, jnp.bfloat16, jnp.uint32
SCOPES = False


def _tables():
    k = np.arange(BK)[None, :]
    n = np.arange(BK)[:, None]
    ang = 2.0 * np.pi * (((4 * k + 1) * n) % (4 * BK)) / (4 * BK)
    ft = np.concatenate([np.cos(ang), np.sin(ang)], axis=1)
    return jnp.asarray(ft, bf16), jnp.asarray(ft.T / BK, bf16)


def _ln(x):
    m = jnp.sum(x, axis=0, keepdims=True) * (1.0 / D)
    xc = x - m
    v = jnp.sum(xc * xc, axis=0, keepdims=True) * (1.0 / D)
    return xc * lax.rsqrt(v + EPS)


def _silu(h):
    t = 0.5 * h
    return t * jnp.tanh(t) + t


def _dot(a, b):
    return jnp.dot(a, b, preferred_element_type=f32)


class _Sc:
    def __init__(self):
        self.c = None
    def __call__(self, name):
        if not SCOPES: return
        if self.c is not None: self.c.__exit__(None, None, None)
        self.c = jax.named_scope(name) if name else None
        if self.c is not None: self.c.__enter__()


def kernel(q_hbm, k_hbm, v_hbm, sh_hbm, h_hbm, d_hbm, w1_hbm, w2t_hbm, ft_hbm, g_hbm, o_hbm,
           q_v, k_v, v_v, h_v, sh_v, d_v, w1_v, w2t_v, w1p_v, w2p_v, ft_v, g_v, col_v, zero_v, zs_ref,
           y_v, x2_v, xn0_v, x30_v, t0_v, dum_v, o_v, sem, wsem, qsem, osem, *grp):
    u_v, hp_v, hraw_v, part_v, yf_v = (grp[i * NG:(i + 1) * NG] for i in range(5))
    sc = _Sc()

    def quad_copies(s):
        cols = pl.ds(pl.multiple_of(s * T, T), T)
        return [pltpu.make_async_copy(src.at[:, cols], dst.at[:, cols], qsem.at[4 * s + i])
                for i, (src, dst) in enumerate(((k_hbm, k_v), (v_hbm, v_v), (h_hbm, h_v), (q_hbm, q_v)))]

    fc = F // W1C
    def w1_copy(c):
        return pltpu.make_async_copy(w1_hbm.at[:, pl.ds(c * fc, fc)], w1_v.at[:, pl.ds(c * fc, fc)], wsem.at[c])

    def out_copy(c0, w, i):
        cols = pl.ds(c0, w)
        return pltpu.make_async_copy(o_v.at[:, cols], o_hbm.at[:, cols], osem.at[i])

    c_sh = pltpu.make_async_copy(sh_hbm, sh_v, sem.at[0])
    c_d = pltpu.make_async_copy(d_hbm, d_v, sem.at[1])
    c_w2 = pltpu.make_async_copy(w2t_hbm, w2t_v, sem.at[2])
    c_ft = pltpu.make_async_copy(ft_hbm, ft_v, sem.at[3])
    c_g = pltpu.make_async_copy(g_hbm, g_v, sem.at[4])
    c_sh.start(); c_d.start(); c_ft.start(); c_g.start()
    cps0 = quad_copies(0)
    for c in cps0[:3]: c.start()

    sc('init')
    for g in range(NG):
        part_v[g][...] = jnp.zeros(part_v[g].shape, f32)
        u_v[g][NB:] = jnp.zeros((Q, RG, 2 * BK), f32)
    zero_v[...] = jnp.zeros(zero_v.shape, jnp.int32)
    zs_ref[0] = 0
    c_sh.wait(); c_d.wait()
    sh = sh_v[...].astype(f32)
    dd = d_v[...].astype(f32).reshape(1, D)
    for t in range(5):
        row = sh[t:t + 1, :] if t < 4 else dd
        col_v[t] = jnp.broadcast_to(row, (128, D)).T

    NRC = RG // RC

    class Conv:
        def __init__(self, q, first):
            self.q, self.first = q, first
            self.cols = pl.ds(0, T) if first else pl.ds(pl.multiple_of(q * T, T), T)
            if not first:
                self.keep = zero_v[...] == 0
            self.prev = {}
            self.kv = [None] * NG
            self.y = [None] * NG

        @staticmethod
        def stack(x):
            w = x.shape[1] // Q
            return jnp.concatenate([x[c * RC:(c + 1) * RC, j * w:(j + 1) * w]
                                    for c in range(NRC) for j in range(Q)], axis=0)

        @staticmethod
        def piece(res, c, j):
            return res[(c * Q + j) * RC:(c * Q + j + 1) * RC]

        def fwd_h(self, g):
            q, first = self.q, self.first
            res = _dot(self.stack(h_v[pl.ds(g * RG, RG), self.cols]), ft_v[...])
            for c in range(NRC):
                r = pl.ds(c * RC, RC)
                for j in range(Q):
                    cur = self.piece(res, c, j)
                    if j == 0 and first:
                        hp_v[g][0, r, :] = cur
                        continue
                    prev = hraw_v[g][r, :] if j == 0 else self.piece(res, c, j - 1)
                    hp_v[g][Q * q + j, r, :BK] = cur[:, :BK] + prev[:, BK:]
                    hp_v[g][Q * q + j, r, BK:] = cur[:, BK:] - prev[:, :BK]
                hraw_v[g][r, :] = self.piece(res, c, Q - 1)

        def fwd_u(self, g):
            q, first = self.q, self.first
            kvs = []
            for c in range(NRC):
                r = pl.ds(g * RG + c * RC, RC)
                if first:
                    kk = jnp.concatenate([jnp.zeros((RC, BK), f32), k_v[r, 0:T].astype(f32)], axis=1)
                else:
                    kk = k_v[r, pl.ds(pl.multiple_of(q * T - BK, BK), T + BK)].astype(f32)
                def col(t):
                    return jnp.tile(col_v[t, r, :], (1, Q))
                ks = kk[:, BK:] * col(0)
                for tau in range(1, 4):
                    ks = ks + pltpu.roll(kk, tau, 1)[:, BK:] * col(tau)
                kvs.append((ks * v_v[r, self.cols].astype(f32)).astype(bf16))
            kv = jnp.concatenate(kvs, axis=0)
            self.kv[g] = kv
            res = _dot(self.stack(kv), ft_v[...])
            for c in range(NRC):
                for j in range(Q):
                    u_v[g][Q * q + j, pl.ds(c * RC, RC), :] = self.piece(res, c, j)

        def chain(self, name, g, pr, init, terms):
            ar = ai = None
            if init is not None:
                ar, ai = init
            prev = None if self.first else self.prev.get(name)
            if prev is not None and ar is not None:
                ar = jnp.where(self.keep, ar, prev[0]); ai = jnp.where(self.keep, ai, prev[1])
                prev = None
            for (j, m) in terms:
                ur = u_v[g][j, pr, :BK]; ui = u_v[g][j, pr, BK:]
                hr = hp_v[g][m, pr, :BK]; hi = hp_v[g][m, pr, BK:]
                if ar is None:
                    ar = ur * hr; ai = ur * hi
                    if prev is not None:
                        ar = jnp.where(self.keep, ar, prev[0]); ai = jnp.where(self.keep, ai, prev[1])
                    ar = ar - ui * hi; ai = ai + ui * hr
                elif self.first:
                    ar = ar + (ur * hr - ui * hi); ai = ai + (ur * hi + ui * hr)
                else:
                    ar = (ar + ur * hr) - ui * hi
                    ai = (ai + ur * hi) + ui * hr
            self.prev[name] = (ar, ai)
            return ar, ai

        def mac(self, g):
            q = self.q
            for p in range(PG):
                pr = pl.ds(p * 8, 8)
                for a in range(Q):
                    terms = [(Q * q + b, a - b) for b in range(a + 1)]
                    init = None
                    if not self.first:
                        init = (part_v[g][a, pr, :BK], part_v[g][a, pr, BK:])
                        terms = [(b, Q * q + a - b) for b in range(Q)] + terms
                    ar, ai = self.chain("c", g, pr, init, terms)
                    yf_v[g][a, pr, :BK] = ar
                    yf_v[g][a, pr, BK:] = ai

        def mac_ahead(self, g):
            q = self.q
            z = zs_ref[0]
            j2 = jnp.where(q == 1, NB, Q)
            m2 = jnp.where(q == 1, Q, 2 * Q) + z
            j1 = Q * q + z
            m1 = Q + z
            for p in range(PG):
                pr = pl.ds(p * 8, 8)
                for a in range(Q):
                    terms = ([(j2 + b, m2 + a - b) for b in range(Q)]
                             + [(j1 + b, m1 + a - b) for b in range(Q)])
                    ar, ai = self.chain("b", g, pr, None, terms)
                    part_v[g][a, pr, :BK] = ar
                    part_v[g][a, pr, BK:] = ai

        def inv(self, g):
            lhs = jnp.concatenate([yf_v[g][j, pl.ds(c * RC, RC), :] for c in range(NRC) for j in range(Q)],
                                  axis=0).astype(bf16)
            res = _dot(lhs, g_v[...])
            conv = jnp.concatenate(
                [jnp.concatenate([self.piece(res, c, j) for j in range(Q)], axis=1) for c in range(NRC)], axis=0)
            dcol = jnp.tile(col_v[4, pl.ds(g * RG, RG), :], (1, Q))
            self.y[g] = conv + self.kv[g].astype(f32) * dcol

        def ytile(self, t):
            return jnp.concatenate([self.y[g][:, t * BK:(t + 1) * BK] for g in range(NG)], axis=0)

    def tie(val, keep, deps):
        head = val[0:8]
        for d in deps:
            head = jnp.where(keep, head, d)
        return jnp.concatenate([head, val[8:]], axis=0)

    def stage(x, y, keep=None, deps=()):
        x = x + _ln(x) * y
        xn = _ln(x)
        if deps: xn = tie(xn, keep, deps)
        return x, xn.astype(bf16), xn[D - 8:]

    def mm1(xn, keep=None, deps=()):
        g = _silu(_dot(pltpu.bitcast(w1p_v[...], bf16), xn))
        if deps: g = tie(g, keep, deps)
        return g.astype(bf16)

    def mm2(x, g):
        return x + _dot(pltpu.bitcast(w2p_v[...], bf16), g)

    def finish_l1(t, x2, y):
        tc = slice(t * BK, (t + 1) * BK)
        if t == 0:
            t0_v[0] = x2
            t0_v[1] = y
        else:
            y_v[:, tc] = y
            x2_v[:, tc] = x2

    def pre_l2():
        z = zs_ref[0]
        x3, xn, last = stage(t0_v[z], t0_v[z + 1])
        xn0_v[...] = pltpu.bitcast(xn, u32)
        x30_v[...] = x3
        return last

    def start_l2(t):
        tc = slice(t * BK, (t + 1) * BK)
        if t == 0:
            return x30_v[...], pltpu.bitcast(xn0_v[...], bf16)
        return stage(x2_v[:, tc], y_v[:, tc])[:2]

    sc('wait_kvh')
    c_ft.wait(); c_g.wait()
    for c in cps0[:3]: c.wait()
    w1_copy(0).start()
    cps0[3].start()
    for c in range(1, W1C): w1_copy(c).start()
    c_w2.start()
    sc('conv0')
    cv = Conv(0, True)
    for g in range(NG):
        cv.fwd_h(g); cv.fwd_u(g)
    for g in range(NG):
        cv.mac(g)
        cv.inv(g)
    sc('wait_w1a')
    w1_copy(0).wait()
    cps0[3].wait()
    sc('mm1a')
    xs, xns, ys = [], [], []
    for t in range(Q):
        y = cv.ytile(t)
        x, xn, _ = stage(q_v[:, t * BK:(t + 1) * BK].astype(f32), y)
        xs.append(x); xns.append(xn); ys.append(y)
    gs = [[] for _ in range(Q)]
    for c in range(W1C):
        if c > 0:
            sc('wait_w1b')
            w1_copy(c).wait()
            sc('mm1b')
        wt = w1_v[:, c * fc:(c + 1) * fc].T
        w1p_v[c * fc // 2:(c + 1) * fc // 2, :] = pltpu.bitcast(wt, u32)
        for t in range(Q):
            gs[t].append(_silu(_dot(wt, xns[t])).astype(bf16))
    sc('wait_w2')
    c_w2.wait()
    for c in quad_copies(1): c.start()
    sc('mm2')
    w2t = w2t_v[...]
    w2p_v[...] = pltpu.bitcast(w2t, u32)
    keep0 = zero_v[...] == 0
    last = None
    for t in range(Q):
        gt = jnp.concatenate(gs[t], axis=0)
        if t == Q - 1:
            gt = jnp.concatenate([tie(gt[0:16].astype(f32), keep0, [pre_l2()]).astype(bf16), gt[16:]], axis=0)
        finish_l1(t, xs[t] + _dot(w2t, gt), ys[t])

    def step(s, carry):
        for c in quad_copies(s + 1): c.wait()
        @pl.when(s + 2 < NS)
        def _():
            for c in quad_copies(s + 2): c.start()
        c_dum = pltpu.make_async_copy(sh_hbm, dum_v, sem.at[5])
        c_dum.start()
        cv = Conv(s + 1, False)
        o0 = pl.multiple_of(s * T, T)
        q0 = pl.multiple_of((s + 1) * T, T)
        def fwd(g):
            cv.fwd_h(g); cv.fwd_u(g); cv.mac(g)
        for t in range(Q):
            x, xn = start_l2(t)
            g = mm1(xn)
            if t < 2: fwd(2 * t)
            if t == Q - 1:
                for gg in range(NG): cv.inv(gg)
            o = mm2(x, g)
            o_v[:, pl.ds(o0 + t * BK, BK)] = o.astype(bf16)
            if t < 2: fwd(2 * t + 1)
        y0 = cv.ytile(0)
        st0 = stage(q_v[:, pl.ds(q0, BK)].astype(f32), y0)
        c_dum.wait()
        for g in range(NG): cv.mac_ahead(g)
        for t in range(Q):
            y = cv.ytile(t)
            fin = t == Q - 1
            x, xn, _ = st0 if t == 0 else stage(q_v[:, pl.ds(q0 + t * BK, BK)].astype(f32), y)
            finish_l1(t, mm2(x, mm1(xn, cv.keep, [pre_l2()] if fin else ())), y)
        out_copy(o0, T, s).start()
        return carry
    sc('loop')
    lax.fori_loop(0, NS - 1, step, 0)

    sc('epi')
    for t in range(Q):
        x, xn = start_l2(t)
        c0 = (NS - 1) * T + t * BK
        o_v[:, c0:c0 + BK] = mm2(x, mm1(xn)).astype(bf16)
        out_copy(c0, BK, NS - 1 + t).start()
    sc('wait_out')
    for s in range(NS - 1):
        out_copy(s * T, T, s).wait()
    for t in range(Q):
        out_copy((NS - 1) * T + t * BK, BK, NS - 1 + t).wait()
    sc(None)


@jax.jit
def pallas_interleave_layers__ssm_conv_h3__dense_activation_silu__prompt_kernel(
        A_q, A_k, A_v, A_shift_k, A_ssm_k, A_ssm_D, B_x, B_w1, B_w2):
    ft, g = _tables()
    anyspec = pl.BlockSpec(memory_space=pl.ANY)
    act = pltpu.VMEM((D, S), bf16)
    grp = ([pltpu.VMEM((NB + Q, RG, 2 * BK), f32)] * NG + [pltpu.VMEM((NB, RG, 2 * BK), f32)] * NG
           + [pltpu.VMEM((RG, 2 * BK), f32)] * NG + [pltpu.VMEM((Q, RG, 2 * BK), f32)] * (2 * NG))
    out = pl.pallas_call(
        kernel,
        in_specs=[anyspec] * 10,
        out_specs=anyspec,
        out_shape=jax.ShapeDtypeStruct((D, S), bf16),
        scratch_shapes=[act, act, act, act, pltpu.VMEM((4, D), bf16), pltpu.VMEM((D,), bf16),
                        pltpu.VMEM((D, F), bf16), pltpu.VMEM((D, F), bf16),
                        pltpu.VMEM((F // 2, D), u32), pltpu.VMEM((D // 2, F), u32),
                        pltpu.VMEM((BK, 2 * BK), bf16), pltpu.VMEM((2 * BK, BK), bf16),
                        pltpu.VMEM((5, D, 128), f32), pltpu.VMEM((8, 128), jnp.int32), pltpu.SMEM((1,), jnp.int32),
                        pltpu.VMEM((D, T), f32), pltpu.VMEM((D, T), f32), pltpu.VMEM((D // 2, BK), u32), pltpu.VMEM((D, BK), f32), pltpu.VMEM((2, D, BK), f32), pltpu.VMEM((4, D), bf16), act,
                        pltpu.SemaphoreType.DMA((6,)), pltpu.SemaphoreType.DMA((W1C,)),
                        pltpu.SemaphoreType.DMA((4 * NS,)), pltpu.SemaphoreType.DMA((NS - 1 + Q,))] + grp,
        compiler_params=pltpu.CompilerParams(vmem_limit_bytes=110 * 1024 * 1024),
    )(A_q[0].T, A_k[0].T, A_v[0].T, A_shift_k.T, A_ssm_k, A_ssm_D, B_w1, B_w2.T, ft, g)
    return out.T[None]
```

```python
import jax
import jax.numpy as jnp
import numpy as np
from jax import lax
import jax.experimental.pallas as pl
import jax.experimental.pallas.tpu as pltpu

S, D, F = 2048, 448, 1792
BK = 128
NB = S // BK
T = 512
Q = T // BK
NS = S // T
W1B = (0, 256, 512, 1024, 1792)
W1C = len(W1B) - 1
RG = 112
NG = D // RG
PG = RG // 8
RC = 16
NRC = RG // RC
EPS = 1e-5
OFFH = 8
PADU = 0
PADH = 16
PADY = 0
f32, bf16, u32 = jnp.float32, jnp.bfloat16, jnp.uint32
SCOPES = False


def _tables():
    k = np.arange(BK)[None, :]
    n = np.arange(BK)[:, None]
    ang = 2.0 * np.pi * (((4 * k + 1) * n) % (4 * BK)) / (4 * BK)
    ft = np.concatenate([np.cos(ang), np.sin(ang)], axis=1)
    return jnp.asarray(ft, bf16), jnp.asarray(ft.T / BK, bf16)


def _ln(x):
    m = jnp.sum(x, axis=0, keepdims=True) * (1.0 / D)
    xc = x - m
    v = jnp.sum(xc * xc, axis=0, keepdims=True) * (1.0 / D)
    return xc * lax.rsqrt(v + EPS)


def _silu(h):
    t = 0.5 * h
    return t * jnp.tanh(t) + t


def _dot(a, b):
    return jnp.dot(a, b, preferred_element_type=f32)


class _Sc:
    def __init__(self):
        self.c = None
    def __call__(self, name):
        if not SCOPES: return
        if self.c is not None: self.c.__exit__(None, None, None)
        self.c = jax.named_scope(name) if name else None
        if self.c is not None: self.c.__enter__()


def kernel(q_hbm, k_hbm, v_hbm, sh_hbm, h_hbm, d_hbm, w1_hbm, w2t_hbm, ft_hbm, g_hbm, o_hbm,
           q_v, k_v, v_v, h_v, sh_v, d_v, w1_v, w2t_v, w1p_v, w2p_v, ft_v, g_v, col_v, zero_v, zs_ref,
           kv_v, y_v, x2_v, gc_v, t3_v, o_v, sem, wsem, fsem, qsem, osem, *grp):
    u_v, hp_v, hraw_v, part_v, yf_v = (grp[i * NG:(i + 1) * NG] for i in range(5))
    sc = _Sc()

    def quad_copy(s, i, sm):
        cols = pl.ds(pl.multiple_of(s * T, T), T)
        src, dst = ((k_hbm, k_v), (v_hbm, v_v), (h_hbm, h_v), (q_hbm, q_v))[i]
        return pltpu.make_async_copy(src.at[:, cols], dst.at[:, cols], sm)

    def quad_copies(s):
        return [quad_copy(s, i, qsem.at[s - 1]) for i in range(4)]

    def w1_copy(c):
        cols = pl.ds(W1B[c], W1B[c + 1] - W1B[c])
        return pltpu.make_async_copy(w1_hbm.at[:, cols], w1_v.at[:, cols], wsem.at[c])

    def half_copy(name, hh, sm):
        at = (pl.ds(hh * 2 * RG, 2 * RG), pl.ds(0, T))
        src, dst = {"k": (k_hbm, k_v), "v": (v_hbm, v_v), "h": (h_hbm, h_v)}[name]
        return pltpu.make_async_copy(src.at[at], dst.at[at], sm)

    def out_copy(c0, w, i):
        cols = pl.ds(c0, w)
        return pltpu.make_async_copy(o_v.at[:, cols], o_hbm.at[:, cols], osem.at[i])

    wave = [[pltpu.make_async_copy(sh_hbm, sh_v, fsem.at[0]), pltpu.make_async_copy(d_hbm, d_v, fsem.at[0])],
            [pltpu.make_async_copy(ft_hbm, ft_v, fsem.at[1]), half_copy("k", 0, fsem.at[1]), half_copy("v", 0, fsem.at[1])],
            [half_copy("h", 0, fsem.at[2]), half_copy("k", 1, fsem.at[2]), half_copy("v", 1, fsem.at[2])],
            [half_copy("h", 1, fsem.at[3]), pltpu.make_async_copy(g_hbm, g_v, fsem.at[3])]]
    c_q0 = quad_copy(0, 3, sem.at[1])
    c_w2 = pltpu.make_async_copy(w2t_hbm, w2t_v, sem.at[2])
    for w in wave[:3]:
        for c in w: c.start()
    zero_v[...] = jnp.zeros(zero_v.shape, jnp.int32)
    zs_ref[0] = 0

    def piece(res, c, j):
        return res[(c * Q + j) * RC:(c * Q + j + 1) * RC]

    def stack(x):
        w = x.shape[1] // Q
        return jnp.concatenate([x[c * RC:(c + 1) * RC, j * w:(j + 1) * w]
                                for c in range(NRC) for j in range(Q)], axis=0)

    class Conv:
        def __init__(self, q, first):
            self.q, self.first = q, first
            self.cols = pl.ds(0, T) if first else pl.ds(pl.multiple_of(q * T, T), T)
            self.keep = zero_v[...] == 0
            self.prev = None
            self.link = not first

        def anchor(self, val, chained=False):
            if chained and self.prev is not None:
                self.prev = tuple(jnp.where(self.keep, p, val) for p in self.prev)
            else:
                self.prev = (val, val)

        def fwd_h(self, g):
            q, first = self.q, self.first
            res = _dot(stack(h_v[pl.ds(g * RG, RG), self.cols]), ft_v[...])
            for c in range(NRC):
                r = pl.ds(c * RC, RC)
                rh = pl.ds(c * RC + OFFH, RC)
                for j in range(Q):
                    cur = piece(res, c, j)
                    if j == 0 and first:
                        hp_v[g][0, rh, :] = cur
                        continue
                    prev = hraw_v[g][r, :] if j == 0 else piece(res, c, j - 1)
                    hp_v[g][Q * q + j, rh, :BK] = cur[:, :BK] + prev[:, BK:]
                    hp_v[g][Q * q + j, rh, BK:] = cur[:, BK:] - prev[:, :BK]
                hraw_v[g][r, :] = piece(res, c, Q - 1)

        def fwd_u(self, g):
            q, first = self.q, self.first
            kvs = []
            for c in range(NRC):
                r = pl.ds(g * RG + c * RC, RC)
                if first:
                    kk = jnp.concatenate([jnp.zeros((RC, BK), f32), k_v[r, 0:T].astype(f32)], axis=1)
                else:
                    kk = k_v[r, pl.ds(pl.multiple_of(q * T - BK, BK), T + BK)].astype(f32)
                def col(t):
                    return jnp.tile(col_v[t, r, :], (1, Q))
                ks = kk[:, BK:] * col(0)
                for tau in range(1, 4):
                    ks = ks + pltpu.roll(kk, tau, 1)[:, BK:] * col(tau)
                kv = (ks * v_v[r, self.cols].astype(f32)).astype(bf16)
                kv_v[pl.ds((g * RG + c * RC) // 2, RC // 2), :] = pltpu.bitcast(kv, u32)
                kvs.append(kv)
            res = _dot(stack(jnp.concatenate(kvs, axis=0)), ft_v[...])
            for c in range(NRC):
                for j in range(Q):
                    u_v[g][Q * q + j, pl.ds(c * RC, RC), :] = piece(res, c, j)
            return res[Q * RG - 8:, BK:]

        def chain(self, g, pr, init, terms):
            ar = ai = None
            if init is not None:
                ar, ai = init
            prev = self.prev if self.link else None
            if prev is not None and ar is not None:
                ar = jnp.where(self.keep, ar, prev[0]); ai = jnp.where(self.keep, ai, prev[1])
                prev = None
            for (j, m) in terms:
                ur = u_v[g][j, pr, :BK]; ui = u_v[g][j, pr, BK:]
                ph = pl.ds(pr.start + OFFH, 8)
                hr = hp_v[g][m, ph, :BK]; hi = hp_v[g][m, ph, BK:]
                if ar is None:
                    ar = ur * hr; ai = ur * hi
                    if prev is not None:
                        ar = jnp.where(self.keep, ar, prev[0]); ai = jnp.where(self.keep, ai, prev[1])
                    ar = ar - ui * hi; ai = ai + ui * hr
                elif self.first:
                    ar = ar + (ur * hr - ui * hi); ai = ai + (ur * hi + ui * hr)
                else:
                    ar = (ar + ur * hr) - ui * hi
                    ai = (ai + ur * hi) + ui * hr
            self.prev = (ar, ai)
            return ar, ai

        def mac(self, p0, p1):
            q = self.q
            for pp in range(p0, p1):
                g, p = divmod(pp, PG)
                pr = pl.ds(p * 8, 8)
                for a in range(Q):
                    terms = [(Q * q + b, a - b) for b in range(a + 1)]
                    init = None
                    if not self.first:
                        init = (part_v[g][a, pr, :BK], part_v[g][a, pr, BK:])
                        terms = [(b, Q * q + a - b) for b in range(Q)] + terms
                    ar, ai = self.chain(g, pr, init, terms)
                    yf_v[g][a, pr, :BK] = ar
                    yf_v[g][a, pr, BK:] = ai

        def mac_ahead(self, p0, p1):
            q = self.q
            j2 = jnp.where(q == 1, NB, Q)
            m2 = jnp.where(q == 1, Q, 2 * Q)
            for pp in range(p0, p1):
                g, p = divmod(pp, PG)
                pr = pl.ds(p * 8, 8)
                for a in range(Q):
                    terms = ([(j2 + b, m2 + a - b) for b in range(Q)]
                             + [(Q * q + b, Q + a - b) for b in range(Q)])
                    ar, ai = self.chain(g, pr, None, terms)
                    part_v[g][a, pr, :BK] = ar
                    part_v[g][a, pr, BK:] = ai

        def inv(self, t):
            halves = []
            for hh in range(2):
                lhs = jnp.concatenate([yf_v[g][t, :RG] for g in (2 * hh, 2 * hh + 1)], axis=0).astype(bf16)
                halves.append(_dot(lhs, g_v[...]))
            kv = pltpu.bitcast(kv_v[:, t * BK:(t + 1) * BK], bf16).astype(f32)
            return jnp.concatenate(halves, axis=0) + kv * col_v[4]

        def inv_group(self, g):
            lhs = jnp.concatenate([yf_v[g][j, :RG] for j in range(Q)], axis=0).astype(bf16)
            res = _dot(lhs, g_v[...])
            kv = pltpu.bitcast(kv_v[g * RG // 2:(g + 1) * RG // 2, :], bf16).astype(f32)
            dcol = col_v[4, g * RG:(g + 1) * RG, :]
            for j in range(Q):
                y = res[j * RG:(j + 1) * RG] + kv[:, j * BK:(j + 1) * BK] * dcol
                y_v[g * RG:(g + 1) * RG, j * BK:(j + 1) * BK] = y

    def split():
        def body(i, c):
            zero_v[...] = jnp.zeros(zero_v.shape, jnp.int32)
            return c
        lax.fori_loop(0, zs_ref[0], body, 0)

    def tie(val, keep, deps):
        head = val[0:8]
        for d in deps:
            head = jnp.where(keep, head, d)
        return jnp.concatenate([head, val[8:]], axis=0)

    def stage(x, y):
        x = x + _ln(x) * y
        xn = _ln(x)
        return x, xn.astype(bf16), xn[D - 8:]

    def mm1(xn):
        return _silu(_dot(pltpu.bitcast(w1p_v[...], bf16), xn))

    def dot2(w, g):
        k0 = 2 * BK
        head = jnp.concatenate([_dot(w[:D // 2, :k0], g[:k0]), _dot(w[D // 2:, :k0], g[:k0])], axis=0)
        return head + _dot(w[:, k0:], g[k0:])

    def mm2(x, g):
        return x + dot2(pltpu.bitcast(w2p_v[...], bf16), g.astype(bf16))

    def finish_l1(t, x2, y):
        tc = slice(t * BK, (t + 1) * BK)
        y_v[:, tc] = y
        x2_v[:, tc] = x2

    def hold_l1(x1, g):
        gc_v[...] = pltpu.bitcast(g.astype(bf16), u32)
        t3_v[...] = x1

    def start_l2(t, keep=None, after=None):
        tc = slice(t * BK, (t + 1) * BK)
        x, y = x2_v[:, tc], y_v[:, tc]
        if after is not None:
            x = tie(x, keep, [after])
        return stage(x, y)

    cv = Conv(0, True)
    sc('wait0')
    for c in wave[0]: c.wait()
    sc('cols')
    sh = sh_v[...].astype(f32)
    dd = d_v[...].astype(f32).reshape(1, D)
    for t in range(5):
        row = sh[t:t + 1, :] if t < 4 else dd
        col_v[t] = jnp.broadcast_to(row, (128, D)).T
    sc('wait1')
    for c in wave[1]: c.wait()
    for c in wave[3]: c.start()
    c_q0.start()
    sc('u01')
    cv.fwd_u(0); cv.fwd_u(1)
    sc('wait2')
    for c in wave[2]: c.wait()
    w1_copy(0).start(); w1_copy(1).start(); w1_copy(2).start()
    sc('u23')
    cv.fwd_u(2); cv.fwd_h(0); cv.fwd_u(3); cv.fwd_h(1)
    sc('wait3')
    for c in wave[3]: c.wait()
    w1_copy(3).start()
    sc('h23')
    cv.fwd_h(2); cv.fwd_h(3)
    cv.link = True
    for g in range(2):
        cv.prev = None; cv.mac(g * PG, (g + 1) * PG)
    cv.link = False
    cv.inv_group(0); cv.inv_group(1)

    def transpose_w1(c):
        wt = w1_v[:, W1B[c]:W1B[c + 1]].T
        w1p_v[W1B[c] // 2:W1B[c + 1] // 2, :] = pltpu.bitcast(wt, u32)

    def ytile(t):
        return y_v[:, t * BK:(t + 1) * BK]

    def w1rows(c0, c1):
        return pltpu.bitcast(w1p_v[W1B[c0] // 2:W1B[c1] // 2, :], bf16)

    sc('wait_q')
    c_q0.wait()
    w1_copy(0).wait()
    c_w2.start()
    sc('st0')
    cv.mac(2 * PG, 4 * PG)
    cv.inv_group(2); cv.inv_group(3)
    transpose_w1(0)
    xs, xns = [None] * Q, [None] * Q
    xs[0], xns[0], _ = stage(q_v[:, 0:BK].astype(f32), ytile(0))
    gs = [[] for _ in range(Q)]
    sc('wait_w1')
    w1_copy(1).wait(); w1_copy(2).wait()
    sc('mm1')
    transpose_w1(1)
    for t in range(Q):
        if t > 0:
            xs[t], xns[t], _ = stage(q_v[:, t * BK:(t + 1) * BK].astype(f32), ytile(t))
        gs[t].append(_silu(_dot(w1rows(0, 1), xns[t])).astype(bf16))
        gs[t].append(_silu(_dot(w1rows(1, 2), xns[t])).astype(bf16))
    transpose_w1(2)
    sc('wait_w1')
    w1_copy(3).wait()
    sc('mm1')
    for t in range(Q):
        gs[t].append(_silu(_dot(w1rows(2, 3), xns[t])).astype(bf16))
    transpose_w1(3)
    for g in range(NG):
        part_v[g][:, :RG] = jnp.zeros((Q, RG, 2 * BK), f32)
        u_v[g][NB:, :RG] = jnp.zeros((Q, RG, 2 * BK), f32)
    sc('wait_w1')
    c_w2.wait()
    for cp in quad_copies(1): cp.start()
    sc('mm1')
    wt = w1rows(3, 4)
    for t in range(Q - 1):
        gs[t].append(_silu(_dot(wt, xns[t])).astype(bf16))
    w2t = w2t_v[...]
    w2p_v[...] = pltpu.bitcast(w2t, u32)
    for t in range(Q - 1):
        x2_v[:, t * BK:(t + 1) * BK] = xs[t] + dot2(w2t, jnp.concatenate(gs[t], axis=0))
    gs[Q - 1].append(_silu(_dot(wt, xns[Q - 1])).astype(bf16))
    hold_l1(xs[Q - 1], jnp.concatenate(gs[Q - 1], axis=0))

    def step(s, carry):
        for c in quad_copies(s + 1): c.wait()
        @pl.when(s + 2 < NS)
        def _():
            for c in quad_copies(s + 2): c.start()
        cv = Conv(s + 1, False)
        o0 = pl.multiple_of(s * T, T)
        q0 = pl.multiple_of((s + 1) * T, T)
        w2 = pltpu.bitcast(w2p_v[...], bf16)
        gc = pltpu.bitcast(gc_v[...], bf16)
        cv.fwd_h(0); cv.fwd_h(1)
        cv.fwd_u(0); cv.fwd_h(2)
        cv.fwd_u(1); cv.fwd_h(3)
        cv.fwd_u(2); acc = t3_v[...] + _dot(w2[:, 0:2 * BK], gc[0:2 * BK])
        after = cv.fwd_u(3); acc = acc + _dot(w2[:, 2 * BK:4 * BK], gc[2 * BK:4 * BK])
        x2_v[:, (Q - 1) * BK:] = acc + dot2(w2[:, 4 * BK:], gc[4 * BK:])
        nxt = start_l2(0, cv.keep, after)
        split()
        cb = (0, 14, 34, 54, 56)
        bb = (0, 2, 19, 35, 51, 56)
        for t in range(Q):
            x, xn, last = nxt
            g = mm1(xn)
            cv.anchor(last if t > 0 else g[0:8])
            cv.mac(cb[t], cb[t + 1])
            if t == Q - 1:
                cv.mac_ahead(bb[0], bb[1])
            if t < Q - 1:
                nxt = start_l2(t + 1, cv.keep, g[F - 8:])
                o_v[:, pl.ds(o0 + t * BK, BK)] = mm2(x, g).astype(bf16)
        g = g.astype(bf16)
        split()
        cv.keep = zero_v[...] == 0
        y = cv.inv(0)
        o_v[:, pl.ds(o0 + (Q - 1) * BK, BK)] = mm2(x, g).astype(bf16)
        x, xn, last = stage(q_v[:, pl.ds(q0, BK)].astype(f32), y)
        for t in range(Q):
            cv.anchor(last); cv.mac_ahead(bb[t + 1], bb[t + 2])
            g = mm1(xn)
            if t + 1 < Q:
                yn = cv.inv(t + 1)
                finish_l1(t, mm2(x, g), y)
                y = yn
                x, xn, last = stage(q_v[:, pl.ds(q0 + (t + 1) * BK, BK)].astype(f32), y)
            else:
                y_v[:, t * BK:] = y
                hold_l1(x, g)
        out_copy(o0, T, s).start()
        return carry
    sc('loop')
    lax.fori_loop(0, NS - 1, step, 0)

    sc('epi')
    x2_v[:, (Q - 1) * BK:] = mm2(t3_v[...], pltpu.bitcast(gc_v[...], bf16))
    for t in range(Q):
        x, xn, _ = start_l2(t)
        c0 = (NS - 1) * T + t * BK
        o_v[:, c0:c0 + BK] = mm2(x, mm1(xn)).astype(bf16)
        out_copy(c0, BK, NS - 1 + t).start()
    sc('wait_out')
    for s in range(NS - 1):
        out_copy(s * T, T, s).wait()
    for t in range(Q):
        out_copy((NS - 1) * T + t * BK, BK, NS - 1 + t).wait()
    sc(None)


@jax.jit
def pallas_interleave_layers__ssm_conv_h3__dense_activation_silu__prompt_kernel(
        A_q, A_k, A_v, A_shift_k, A_ssm_k, A_ssm_D, B_x, B_w1, B_w2):
    ft, g = _tables()
    anyspec = pl.BlockSpec(memory_space=pl.ANY)
    act = pltpu.VMEM((D, S), bf16)
    grp = ([pltpu.VMEM((NB + Q, RG + PADU, 2 * BK), f32)] * NG + [pltpu.VMEM((NB, RG + PADH, 2 * BK), f32)] * NG
           + [pltpu.VMEM((RG, 2 * BK), f32)] * NG + [pltpu.VMEM((Q, RG + PADY, 2 * BK), f32)] * (2 * NG))
    out = pl.pallas_call(
        kernel,
        in_specs=[anyspec] * 10,
        out_specs=anyspec,
        out_shape=jax.ShapeDtypeStruct((D, S), bf16),
        scratch_shapes=[act, act, act, act, pltpu.VMEM((4, D), bf16), pltpu.VMEM((D,), bf16),
                        pltpu.VMEM((D, F), bf16), pltpu.VMEM((D, F), bf16),
                        pltpu.VMEM((F // 2, D), u32), pltpu.VMEM((D // 2, F), u32),
                        pltpu.VMEM((BK, 2 * BK), bf16), pltpu.VMEM((2 * BK, BK), bf16),
                        pltpu.VMEM((5, D, 128), f32), pltpu.VMEM((8, 128), jnp.int32), pltpu.SMEM((1,), jnp.int32),
                        pltpu.VMEM((D // 2, T), u32),
                        pltpu.VMEM((D, T), f32), pltpu.VMEM((D, T), f32), pltpu.VMEM((F // 2, BK), u32),
                        pltpu.VMEM((D, BK), f32), act,
                        pltpu.SemaphoreType.DMA((3,)), pltpu.SemaphoreType.DMA((W1C,)), pltpu.SemaphoreType.DMA((4,)),
                        pltpu.SemaphoreType.DMA((NS - 1,)), pltpu.SemaphoreType.DMA((NS - 1 + Q,))] + grp,
        compiler_params=pltpu.CompilerParams(vmem_limit_bytes=110 * 1024 * 1024),
    )(A_q[0].T, A_k[0].T, A_v[0].T, A_shift_k.T, A_ssm_k, A_ssm_D, B_w1, B_w2.T, ft, g)
    return out.T[None]
```

```python
import jax
import jax.numpy as jnp
import numpy as np
from jax import lax
import jax.experimental.pallas as pl
import jax.experimental.pallas.tpu as pltpu

S, D, F = 2048, 448, 1792
BK = 128
NB = S // BK
T = 512
Q = T // BK
NS = S // T
W1B = (0, 256, 512, 1024, 1792)
W1C = len(W1B) - 1
RG = 112
NG = D // RG
PG = RG // 8
RC = 16
NRC = RG // RC
EPS = 1e-5
SPLIT0 = bool(1)
SPLIT1 = bool(0)
LINK0 = bool(1)
A0 = 2
STH = 0
MIDK = 6
OFFH = 8
PADU = 0
PADH = 16
PADY = 0
f32, bf16, u32 = jnp.float32, jnp.bfloat16, jnp.uint32
SCOPES = False


def _tables():
    k = np.arange(BK)[None, :]
    n = np.arange(BK)[:, None]
    ang = 2.0 * np.pi * (((4 * k + 1) * n) % (4 * BK)) / (4 * BK)
    ft = np.concatenate([np.cos(ang), np.sin(ang)], axis=1)
    return jnp.asarray(ft, bf16), jnp.asarray(ft.T / BK, bf16)


def _ln(x):
    m = jnp.sum(x, axis=0, keepdims=True) * (1.0 / D)
    xc = x - m
    v = jnp.sum(xc * xc, axis=0, keepdims=True) * (1.0 / D)
    return xc * lax.rsqrt(v + EPS)


def _silu(h):
    t = 0.5 * h
    return t * jnp.tanh(t) + t


def _dot(a, b):
    return jnp.dot(a, b, preferred_element_type=f32)


class _Sc:
    def __init__(self):
        self.c = None
    def __call__(self, name):
        if not SCOPES: return
        if self.c is not None: self.c.__exit__(None, None, None)
        self.c = jax.named_scope(name) if name else None
        if self.c is not None: self.c.__enter__()


def kernel(q_hbm, k_hbm, v_hbm, sh_hbm, h_hbm, d_hbm, w1_hbm, w2t_hbm, ft_hbm, g_hbm, o_hbm,
           q_v, k_v, v_v, h_v, sh_v, d_v, w1_v, w2t_v, w1p_v, w2p_v, ft_v, g_v, col_v, zero_v, zs_ref,
           kv_v, y_v, x2_v, gc_v, t3_v, o_v, sem, wsem, fsem, qsem, osem, *grp):
    u_v, hp_v, hraw_v, part_v, yf_v = (grp[i * NG:(i + 1) * NG] for i in range(5))
    sc = _Sc()

    def quad_copy(s, i, sm):
        cols = pl.ds(pl.multiple_of(s * T, T), T)
        src, dst = ((k_hbm, k_v), (v_hbm, v_v), (h_hbm, h_v), (q_hbm, q_v))[i]
        return pltpu.make_async_copy(src.at[:, cols], dst.at[:, cols], sm)

    def quad_copies(s):
        return [quad_copy(s, i, qsem.at[s - 1]) for i in range(4)]

    def w1_copy(c):
        cols = pl.ds(W1B[c], W1B[c + 1] - W1B[c])
        return pltpu.make_async_copy(w1_hbm.at[:, cols], w1_v.at[:, cols], wsem.at[c])

    def half_copy(name, hh, sm):
        at = (pl.ds(hh * 2 * RG, 2 * RG), pl.ds(0, T))
        src, dst = {"k": (k_hbm, k_v), "v": (v_hbm, v_v), "h": (h_hbm, h_v)}[name]
        return pltpu.make_async_copy(src.at[at], dst.at[at], sm)

    def out_copy(c0, w, i):
        cols = pl.ds(c0, w)
        return pltpu.make_async_copy(o_v.at[:, cols], o_hbm.at[:, cols], osem.at[i])

    wave = [[pltpu.make_async_copy(sh_hbm, sh_v, fsem.at[0]), pltpu.make_async_copy(d_hbm, d_v, fsem.at[0])],
            [pltpu.make_async_copy(ft_hbm, ft_v, fsem.at[1]), quad_copy(0, 2, fsem.at[1])],
            [half_copy("k", 0, fsem.at[2]), half_copy("v", 0, fsem.at[2])],
            [half_copy("k", 1, fsem.at[3]), half_copy("v", 1, fsem.at[3])]]
    c_g = pltpu.make_async_copy(g_hbm, g_v, sem.at[0])
    c_q0 = quad_copy(0, 3, sem.at[1])
    c_w2 = pltpu.make_async_copy(w2t_hbm, w2t_v, sem.at[2])
    for w in wave[:3]:
        for c in w: c.start()
    zero_v[...] = jnp.zeros(zero_v.shape, jnp.int32)
    zs_ref[0] = 0

    def piece(res, c, j):
        return res[(c * Q + j) * RC:(c * Q + j + 1) * RC]

    def stack(x):
        w = x.shape[1] // Q
        return jnp.concatenate([x[c * RC:(c + 1) * RC, j * w:(j + 1) * w]
                                for c in range(NRC) for j in range(Q)], axis=0)

    class Conv:
        def __init__(self, q, first):
            self.q, self.first = q, first
            self.cols = pl.ds(0, T) if first else pl.ds(pl.multiple_of(q * T, T), T)
            self.keep = zero_v[...] == 0
            self.prev = None
            self.link = not first

        def anchor(self, val, chained=False):
            if chained and self.prev is not None:
                self.prev = tuple(jnp.where(self.keep, p, val) for p in self.prev)
            else:
                self.prev = (val, val)

        def fwd_h(self, g):
            q, first = self.q, self.first
            res = _dot(stack(h_v[pl.ds(g * RG, RG), self.cols]), ft_v[...])
            for c in range(NRC):
                r = pl.ds(c * RC, RC)
                rh = pl.ds(c * RC + OFFH, RC)
                for j in range(Q):
                    cur = piece(res, c, j)
                    if j == 0 and first:
                        hp_v[g][0, rh, :] = cur
                        continue
                    prev = hraw_v[g][r, :] if j == 0 else piece(res, c, j - 1)
                    hp_v[g][Q * q + j, rh, :BK] = cur[:, :BK] + prev[:, BK:]
                    hp_v[g][Q * q + j, rh, BK:] = cur[:, BK:] - prev[:, :BK]
                hraw_v[g][r, :] = piece(res, c, Q - 1)

        def fwd_u(self, g):
            q, first = self.q, self.first
            lhs = []
            for c in range(NRC):
                r = pl.ds(g * RG + c * RC, RC)
                if first:
                    kk = jnp.concatenate([jnp.zeros((RC // 2, BK), u32), pltpu.bitcast(k_v[r, 0:T], u32)], axis=1)
                else:
                    kk = pltpu.bitcast(k_v[r, pl.ds(pl.multiple_of(q * T - BK, BK), T + BK)], u32)
                def col(t):
                    return jnp.tile(col_v[t, r, :], (1, Q))
                def wide(p):
                    return pltpu.bitcast(p[:, BK:], bf16).astype(f32)
                ks = wide(kk) * col(0)
                for tau in range(1, 4):
                    ks = ks + wide(pltpu.roll(kk, tau, 1)) * col(tau)
                kv = ks * v_v[r, self.cols].astype(f32)
                for j in range(Q):
                    b = pltpu.bitcast(kv[:, j * BK:(j + 1) * BK].astype(bf16), u32)
                    kv_v[pl.ds((g * RG + c * RC) // 2, RC // 2), j * BK:(j + 1) * BK] = b
                    lhs.append(b)
            res = _dot(pltpu.bitcast(jnp.concatenate(lhs, axis=0), bf16), ft_v[...])
            for c in range(NRC):
                for j in range(Q):
                    u_v[g][Q * q + j, pl.ds(c * RC, RC), :] = piece(res, c, j)
            return res[Q * RG - 8:, BK:]

        def chain(self, g, pr, init, terms):
            ar = ai = None
            if init is not None:
                ar, ai = init
            prev = self.prev if self.link else None
            if prev is not None and ar is not None:
                ar = jnp.where(self.keep, ar, prev[0]); ai = jnp.where(self.keep, ai, prev[1])
                prev = None
            for (j, m) in terms:
                ur = u_v[g][j, pr, :BK]; ui = u_v[g][j, pr, BK:]
                ph = pl.ds(pr.start + OFFH, 8)
                hr = hp_v[g][m, ph, :BK]; hi = hp_v[g][m, ph, BK:]
                if ar is None:
                    ar = ur * hr; ai = ur * hi
                    if prev is not None:
                        ar = jnp.where(self.keep, ar, prev[0]); ai = jnp.where(self.keep, ai, prev[1])
                    ar = ar - ui * hi; ai = ai + ui * hr
                elif self.first:
                    ar = ar + (ur * hr - ui * hi); ai = ai + (ur * hi + ui * hr)
                else:
                    ar = (ar + ur * hr) - ui * hi
                    ai = (ai + ur * hi) + ui * hr
            self.prev = (ar, ai)
            return ar, ai

        def mac(self, p0, p1):
            q = self.q
            for pp in range(p0, p1):
                g, p = divmod(pp, PG)
                pr = pl.ds(p * 8, 8)
                for a in range(Q):
                    terms = [(Q * q + b, a - b) for b in range(a + 1)]
                    init = None
                    if not self.first:
                        init = (part_v[g][a, pr, :BK], part_v[g][a, pr, BK:])
                        terms = [(b, Q * q + a - b) for b in range(Q)] + terms
                    ar, ai = self.chain(g, pr, init, terms)
                    yf_v[g][a, pr, :BK] = ar
                    yf_v[g][a, pr, BK:] = ai

        def mac_ahead(self, p0, p1):
            q = self.q
            j2 = jnp.where(q == 1, NB, Q)
            m2 = jnp.where(q == 1, Q, 2 * Q)
            for pp in range(p0, p1):
                g, p = divmod(pp, PG)
                pr = pl.ds(p * 8, 8)
                for a in range(Q):
                    terms = ([(j2 + b, m2 + a - b) for b in range(Q)]
                             + [(Q * q + b, Q + a - b) for b in range(Q)])
                    ar, ai = self.chain(g, pr, None, terms)
                    part_v[g][a, pr, :BK] = ar
                    part_v[g][a, pr, BK:] = ai

        def inv(self, t):
            halves = []
            for hh in range(2):
                lhs = jnp.concatenate([yf_v[g][t, :RG] for g in (2 * hh, 2 * hh + 1)], axis=0).astype(bf16)
                halves.append(_dot(lhs, g_v[...]))
            kv = pltpu.bitcast(kv_v[:, t * BK:(t + 1) * BK], bf16).astype(f32)
            return jnp.concatenate(halves, axis=0) + kv * col_v[4]

        def inv_group(self, g):
            lhs = jnp.concatenate([yf_v[g][j, :RG] for j in range(Q)], axis=0).astype(bf16)
            res = _dot(lhs, g_v[...])
            kv = pltpu.bitcast(kv_v[g * RG // 2:(g + 1) * RG // 2, :], bf16).astype(f32)
            dcol = col_v[4, g * RG:(g + 1) * RG, :]
            for j in range(Q):
                y = res[j * RG:(j + 1) * RG] + kv[:, j * BK:(j + 1) * BK] * dcol
                y_v[g * RG:(g + 1) * RG, j * BK:(j + 1) * BK] = y

    def split():
        def body(i, c):
            zero_v[...] = jnp.zeros(zero_v.shape, jnp.int32)
            return c
        lax.fori_loop(0, zs_ref[0], body, 0)

    def tie(val, keep, deps):
        head = val[0:8]
        for d in deps:
            head = jnp.where(keep, head, d)
        return jnp.concatenate([head, val[8:]], axis=0)

    def stage(x, y):
        x = x + _ln(x) * y
        xn = _ln(x)
        return x, xn.astype(bf16), xn[D - 8:]

    def mm1(xn):
        return _silu(_dot(pltpu.bitcast(w1p_v[...], bf16), xn))

    def cut(g, ks):
        return [g[a * BK:b * BK].astype(bf16) for a, b in zip(ks[:-1], ks[1:])]

    def head2(w, g0):
        return jnp.concatenate([_dot(w[:D // 2], g0), _dot(w[D // 2:], g0)], axis=0)

    def dot2(w, g):
        g0, g1 = cut(g, (0, 2, g.shape[0] // BK))
        return head2(w[:, :2 * BK], g0) + _dot(w[:, 2 * BK:], g1)

    def mm2(x, g):
        return x + dot2(pltpu.bitcast(w2p_v[...], bf16), g)

    KS = (0, 2, MIDK, F // BK)

    def mm2_mid(x, gpieces):
        w = pltpu.bitcast(w2p_v[...], bf16)
        g0, g1, g2 = gpieces
        k0, k1 = 2 * BK, MIDK * BK
        mid = head2(w[:, :k0], g0) + _dot(w[:, k0:k1], g1)
        return x + (mid + _dot(w[:, k1:], g2)), mid[D - 8:]

    def finish_l1(t, x2, y):
        tc = slice(t * BK, (t + 1) * BK)
        y_v[:, tc] = y
        x2_v[:, tc] = x2

    def hold_l1(x1, g):
        gc_v[...] = pltpu.bitcast(g.astype(bf16), u32)
        t3_v[...] = x1

    def start_l2(t, keep=None, after=None):
        tc = slice(t * BK, (t + 1) * BK)
        x, y = x2_v[:, tc], y_v[:, tc]
        if after is not None:
            x = tie(x, keep, [after])
        return stage(x, y)

    cv = Conv(0, True)
    sc('wait0')
    for c in wave[0]: c.wait()
    sc('cols')
    sh = sh_v[...].astype(f32)
    dd = d_v[...].astype(f32).reshape(1, D)
    for t in range(5):
        row = sh[t:t + 1, :] if t < 4 else dd
        col_v[t] = jnp.broadcast_to(row, (128, D)).T
    sc('wait1')
    for c in wave[1]: c.wait()
    c_g.start()
    for c in wave[3]: c.start()
    c_q0.start()
    sc('h')
    for g in range(NG): cv.fwd_h(g)
    sc('wait2')
    for c in wave[2]: c.wait()
    w1_copy(0).start(); w1_copy(1).start(); w1_copy(2).start()
    sc('u01')
    cv.fwd_u(0); cv.fwd_u(1)
    sc('waitg')
    c_g.wait()
    sc('m01')
    cv.mac(0, 2 * PG)
    cv.inv_group(0); cv.inv_group(1)
    sc('wait3')
    for c in wave[3]: c.wait()
    w1_copy(3).start()
    sc('u23')
    cv.fwd_u(2); cv.fwd_u(3)

    def transpose_w1(c):
        wt = w1_v[:, W1B[c]:W1B[c + 1]].T
        w1p_v[W1B[c] // 2:W1B[c + 1] // 2, :] = pltpu.bitcast(wt, u32)

    def ytile(t):
        return y_v[:, t * BK:(t + 1) * BK]

    def w1rows(c0, c1):
        return pltpu.bitcast(w1p_v[W1B[c0] // 2:W1B[c1] // 2, :], bf16)

    sc('wait_q')
    c_q0.wait()
    w1_copy(0).wait()
    c_w2.start()
    sc('st0')
    cv.mac(2 * PG, 4 * PG)
    cv.inv_group(2); cv.inv_group(3)
    transpose_w1(0)
    xs, xns = [None] * Q, [None] * Q
    xs[0], xns[0], _ = stage(q_v[:, 0:BK].astype(f32), ytile(0))
    gs = [[] for _ in range(Q)]
    sc('wait_w1')
    w1_copy(1).wait(); w1_copy(2).wait()
    sc('mm1')
    transpose_w1(1); transpose_w1(2)

    def a_part(c, t):
        g = _silu(_dot(w1rows(c, c + 1), xns[t]))
        gs[t].append(g.astype(bf16))
        return g

    keep0 = zero_v[...] == 0
    for t in range(Q):
        for c in range(3 if t < Q - 1 else 2):
            g = a_part(c, t)
            if c == 0 and t + 1 < Q:
                x = tie(q_v[:, (t + 1) * BK:(t + 2) * BK].astype(f32), keep0, [g[0:8]])
                xs[t + 1], xns[t + 1], _ = stage(x, ytile(t + 1))
    sc('wait_w1')
    w1_copy(3).wait()
    sc('mm1')
    transpose_w1(3)
    keep0 = zero_v[...] == 0
    a_part(2, Q - 1)
    pieces = []
    for t in range(Q - 1):
        g = a_part(3, t)
        pieces += [g[i * 8:(i + 1) * 8] for i in range(0, 96, 9)]
    for i in range(2 * NG * Q):
        z = jnp.tile(jnp.where(keep0, 0.0, pieces[i]), (PG, 2))
        g, a = divmod(i % (NG * Q), Q)
        if i < NG * Q:
            part_v[g][a, :RG] = z
        else:
            u_v[g][NB + a, :RG] = z
    sc('wait_w1')
    c_w2.wait()
    for cp in quad_copies(1): cp.start()
    sc('mm1')
    a_part(3, Q - 1)
    for c in range(W1C):
        gc_v[W1B[c] // 2:W1B[c + 1] // 2, :] = pltpu.bitcast(gs[Q - 1][c], u32)
    t3_v[...] = xs[Q - 1]
    w2t = w2t_v[...]
    w2p_v[...] = pltpu.bitcast(w2t, u32)
    for t in range(Q - 1):
        acc = head2(w2t[:, :W1B[1]], gs[t][0])
        for c in range(1, W1C):
            acc = acc + _dot(w2t[:, W1B[c]:W1B[c + 1]], gs[t][c])
        x2_v[:, t * BK:(t + 1) * BK] = xs[t] + acc

    def step(s, carry):
        for c in quad_copies(s + 1): c.wait()
        @pl.when(s + 2 < NS)
        def _():
            for c in quad_copies(s + 2): c.start()
        cv = Conv(s + 1, False)
        o0 = pl.multiple_of(s * T, T)
        q0 = pl.multiple_of((s + 1) * T, T)
        w2 = pltpu.bitcast(w2p_v[...], bf16)
        gc = pltpu.bitcast(gc_v[...], bf16)
        cv.fwd_h(0); cv.fwd_h(1)
        cv.fwd_u(0); cv.fwd_h(2)
        cv.fwd_u(1); cv.fwd_h(3)
        cv.fwd_u(2); acc = t3_v[...] + _dot(w2[:, 0:2 * BK], gc[0:2 * BK])
        after = cv.fwd_u(3); acc = acc + _dot(w2[:, 2 * BK:4 * BK], gc[2 * BK:4 * BK])
        if A0 == 1: after = acc[D - 8:]
        if A0 == 2:
            hd = jnp.concatenate([_dot(w2[:D // 2, 4 * BK:6 * BK], gc[4 * BK:6 * BK]), _dot(w2[D // 2:, 4 * BK:6 * BK], gc[4 * BK:6 * BK])], axis=0)
            after = hd[D - 8:]
            x2_v[:, (Q - 1) * BK:] = acc + hd + _dot(w2[:, 6 * BK:], gc[6 * BK:])
        else:
            x2_v[:, (Q - 1) * BK:] = acc + dot2(w2[:, 4 * BK:], gc[4 * BK:])
        nxt = start_l2(0, cv.keep, after)
        if SPLIT0: split()
        cb = (0, 14, 34, 54, 56)
        bb = (0, 2, 19, 35, 51, 56)
        for t in range(Q):
            x, xn, _ = nxt
            g = mm1(xn)
            if t == 0:
                cv.anchor(g[0:8]); cv.mac(cb[0], cb[1])
            if t < Q - 1:
                o, mid = mm2_mid(x, cut(g, KS))
                nxt = start_l2(t + 1, cv.keep, g[F - 8:])
                o_v[:, pl.ds(o0 + t * BK, BK)] = o.astype(bf16)
                cv.anchor(mid); cv.mac(cb[t + 1], cb[t + 2])
                if t == Q - 2:
                    cv.mac_ahead(bb[0], bb[1])
        g = cut(g, KS)
        if SPLIT1: split()
        cv.keep = zero_v[...] == 0
        y = cv.inv(0)
        o, mid = mm2_mid(x, g)
        o_v[:, pl.ds(o0 + (Q - 1) * BK, BK)] = o.astype(bf16)
        x, xn, _ = stage(q_v[:, pl.ds(q0, BK)].astype(f32), y)
        for t in range(Q):
            cv.anchor(mid); cv.mac_ahead(bb[t + 1], bb[t + 2])
            g = mm1(xn)
            if t + 1 < Q:
                yn = cv.inv(t + 1)
                o, mid = mm2_mid(x, cut(g, KS))
                finish_l1(t, o, y)
                y = yn
                x, xn, _ = stage(q_v[:, pl.ds(q0 + (t + 1) * BK, BK)].astype(f32), y)
            else:
                y_v[:, t * BK:] = y
                hold_l1(x, g)
        out_copy(o0, T, s).start()
        return carry
    sc('loop')
    lax.fori_loop(0, NS - 1, step, 0)

    sc('epi')
    x2_v[:, (Q - 1) * BK:] = mm2(t3_v[...], pltpu.bitcast(gc_v[...], bf16))
    for t in range(Q):
        x, xn, _ = start_l2(t)
        c0 = (NS - 1) * T + t * BK
        o_v[:, c0:c0 + BK] = mm2(x, mm1(xn)).astype(bf16)
        out_copy(c0, BK, NS - 1 + t).start()
    sc('wait_out')
    for s in range(NS - 1):
        out_copy(s * T, T, s).wait()
    for t in range(Q):
        out_copy((NS - 1) * T + t * BK, BK, NS - 1 + t).wait()
    sc(None)


@jax.jit
def pallas_interleave_layers__ssm_conv_h3__dense_activation_silu__prompt_kernel(
        A_q, A_k, A_v, A_shift_k, A_ssm_k, A_ssm_D, B_x, B_w1, B_w2):
    ft, g = _tables()
    anyspec = pl.BlockSpec(memory_space=pl.ANY)
    act = pltpu.VMEM((D, S), bf16)
    grp = ([pltpu.VMEM((NB + Q, RG + PADU, 2 * BK), f32)] * NG + [pltpu.VMEM((NB, RG + PADH, 2 * BK), f32)] * NG
           + [pltpu.VMEM((RG, 2 * BK), f32)] * NG + [pltpu.VMEM((Q, RG + PADY, 2 * BK), f32)] * (2 * NG))
    out = pl.pallas_call(
        kernel,
        in_specs=[anyspec] * 10,
        out_specs=anyspec,
        out_shape=jax.ShapeDtypeStruct((D, S), bf16),
        scratch_shapes=[act, act, act, act, pltpu.VMEM((4, D), bf16), pltpu.VMEM((D,), bf16),
                        pltpu.VMEM((D, F), bf16), pltpu.VMEM((D, F), bf16),
                        pltpu.VMEM((F // 2, D), u32), pltpu.VMEM((D // 2, F), u32),
                        pltpu.VMEM((BK, 2 * BK), bf16), pltpu.VMEM((2 * BK, BK), bf16),
                        pltpu.VMEM((5, D, 128), f32), pltpu.VMEM((8, 128), jnp.int32), pltpu.SMEM((1,), jnp.int32),
                        pltpu.VMEM((D // 2, T), u32),
                        pltpu.VMEM((D, T), f32), pltpu.VMEM((D, T), f32), pltpu.VMEM((F // 2, BK), u32),
                        pltpu.VMEM((D, BK), f32), act,
                        pltpu.SemaphoreType.DMA((3,)), pltpu.SemaphoreType.DMA((W1C,)), pltpu.SemaphoreType.DMA((4,)),
                        pltpu.SemaphoreType.DMA((NS - 1,)), pltpu.SemaphoreType.DMA((NS - 1 + Q,))] + grp,
        compiler_params=pltpu.CompilerParams(vmem_limit_bytes=110 * 1024 * 1024, disable_bounds_checks=True,
                                             disable_semaphore_checks=True),
    )(A_q[0].T, A_k[0].T, A_v[0].T, A_shift_k.T, A_ssm_k, A_ssm_D, B_w1, B_w2.T, ft, g)
    return out.T[None]
```

```python
import jax
import jax.numpy as jnp
import numpy as np
from jax import lax
import jax.experimental.pallas as pl
import jax.experimental.pallas.tpu as pltpu

S, D, F = 2048, 448, 1792
BK = 128
NB = S // BK
T = 512
Q = T // BK
NS = S // T
RG = 112
NG = D // RG
PG = RG // 8
NP = NG * PG
RC = 16
NRC = RG // RC
W1B = (0, 256, 512, 1024, 1792)
W1C = len(W1B) - 1
KS = (0, 2, 6, F // BK)
U0, UC, UP, HL, HW, NSP = 0, 4, 8, 12, 24, 31
HOFF = 8
CB = (0, 14, 34, 54, 56)
BB = (0, 2, 19, 35, 51, 56)
EPS = 1e-5
f32, bf16, u32, i32 = jnp.float32, jnp.bfloat16, jnp.uint32, jnp.int32


def _tables():
    k = np.arange(BK)[None, :]
    n = np.arange(BK)[:, None]
    ang = 2.0 * np.pi * (((4 * k + 1) * n) % (4 * BK)) / (4 * BK)
    fwd = np.concatenate([np.cos(ang), np.sin(ang)], axis=1)
    return jnp.asarray(fwd, bf16), jnp.asarray(fwd.T / BK, bf16)


def _ln(x):
    m = jnp.sum(x, axis=0, keepdims=True) * (1.0 / D)
    xc = x - m
    v = jnp.sum(xc * xc, axis=0, keepdims=True) * (1.0 / D)
    return xc * lax.rsqrt(v + EPS)


def _silu(h):
    t = 0.5 * h
    return t * jnp.tanh(t) + t


def _dot(a, b):
    return jnp.dot(a, b, preferred_element_type=f32)


def _unpack(x):
    return pltpu.bitcast(x, bf16)


def _tile(t):
    return slice(t * BK, (t + 1) * BK)


def _kernel(q_hbm, k_hbm, v_hbm, sh_hbm, h_hbm, d_hbm, w1_hbm, w2t_hbm, ft_hbm, gt_hbm, o_hbm,
            q_v, k_v, v_v, h_v, o_v, sh_v, d_v, w1_v, w2t_v, w1p_v, w2p_v, ft_v, gt_v, col_v, zero_v, zs_ref,
            kv_v, y_v, x2_v, gc_v, x1_v, sem, wsem, qsem, osem, *grp):
    sp_v, hraw_v, part_v, yf_v = (grp[i * NG:(i + 1) * NG] for i in range(4))

    def step_copy(s, i, sm):
        cols = pl.ds(pl.multiple_of(s * T, T), T)
        src, dst = ((k_hbm, k_v), (v_hbm, v_v), (h_hbm, h_v), (q_hbm, q_v))[i]
        return pltpu.make_async_copy(src.at[:, cols], dst.at[:, cols], sm)

    def step_copies(s):
        return [step_copy(s, i, qsem.at[s - 1]) for i in range(4)]

    def half_copies(hh, sm):
        at = (pl.ds(hh * 2 * RG, 2 * RG), pl.ds(0, T))
        return [pltpu.make_async_copy(src.at[at], dst.at[at], sm) for src, dst in ((k_hbm, k_v), (v_hbm, v_v))]

    def w1_copy(c):
        cols = pl.ds(W1B[c], W1B[c + 1] - W1B[c])
        return pltpu.make_async_copy(w1_hbm.at[:, cols], w1_v.at[:, cols], wsem.at[c])

    def out_copy(c0, w):
        cols = pl.ds(c0, w)
        return pltpu.make_async_copy(o_v.at[:, cols], o_hbm.at[:, cols], osem)

    c_taps = [pltpu.make_async_copy(sh_hbm, sh_v, sem.at[0]), pltpu.make_async_copy(d_hbm, d_v, sem.at[0])]
    c_h0 = [pltpu.make_async_copy(ft_hbm, ft_v, sem.at[1]), step_copy(0, 2, sem.at[1])]
    c_kv0 = half_copies(0, sem.at[2])
    c_kv1 = half_copies(1, sem.at[3])
    c_gt = pltpu.make_async_copy(gt_hbm, gt_v, sem.at[4])
    c_q0 = step_copy(0, 3, sem.at[5])
    c_w2 = pltpu.make_async_copy(w2t_hbm, w2t_v, sem.at[6])
    for c in c_taps + c_h0 + c_kv0:
        c.start()
    zero_v[...] = jnp.zeros(zero_v.shape, i32)
    zs_ref[0] = 0

    def all_true():
        return zero_v[...] == 0

    def split():
        def body(i, c):
            zero_v[...] = jnp.zeros(zero_v.shape, i32)
            return c
        lax.fori_loop(0, zs_ref[0], body, 0)

    def tie(val, keep, dep):
        return jnp.concatenate([jnp.where(keep, val[0:8], dep), val[8:]], axis=0)

    def piece(res, c, j):
        return res[(c * Q + j) * RC:(c * Q + j + 1) * RC]

    class Conv:
        def __init__(self, q):
            self.q = q
            self.first = isinstance(q, int)
            self.cols = pl.ds(0, T) if self.first else pl.ds(pl.multiple_of(q * T, T), T)
            self.ub = U0 if self.first else UC
            self.keep = None if self.first else all_true()
            self.prev = None

        def anchor(self, val):
            self.prev = (val, val)

        def fwd_h(self, g):
            hh = h_v[pl.ds(g * RG, RG), self.cols]
            lhs = jnp.concatenate([hh[c * RC:(c + 1) * RC, _tile(j)] for c in range(NRC) for j in range(Q)], axis=0)
            res = _dot(lhs, ft_v[...])
            low = HL + Q * jnp.minimum(self.q, 2)
            for c in range(NRC):
                r = pl.ds(c * RC, RC)
                rh = pl.ds(c * RC + HOFF, RC)
                for j in range(Q):
                    hp = piece(res, c, j)
                    if j > 0 or not self.first:
                        prev = hraw_v[g][r, :] if j == 0 else piece(res, c, j - 1)
                        hp = jnp.concatenate([hp[:, :BK] + prev[:, BK:], hp[:, BK:] - prev[:, :BK]], axis=1)
                    if self.first:
                        sp_v[g][HL + j, rh, :] = hp
                        if j > 0:
                            sp_v[g][HW + j - 1, rh, :] = hp
                    else:
                        sp_v[g][HW + Q - 1 + j, rh, :] = hp
                        sp_v[g][low + j, rh, :] = hp
                hraw_v[g][r, :] = piece(res, c, Q - 1)

        def fwd_u(self, g):
            lhs = []
            for c in range(NRC):
                r = pl.ds(g * RG + c * RC, RC)
                if self.first:
                    kk = jnp.concatenate([jnp.zeros((RC // 2, BK), u32), pltpu.bitcast(k_v[r, 0:T], u32)], axis=1)
                else:
                    kk = pltpu.bitcast(k_v[r, pl.ds(pl.multiple_of(self.q * T - BK, BK), T + BK)], u32)
                ks = None
                for tau in range(4):
                    shifted = kk if tau == 0 else pltpu.roll(kk, tau, 1)
                    term = _unpack(shifted[:, BK:]).astype(f32) * jnp.tile(col_v[tau, r, :], (1, Q))
                    ks = term if ks is None else ks + term
                kv = ks * v_v[r, self.cols].astype(f32)
                for j in range(Q):
                    b = pltpu.bitcast(kv[:, _tile(j)].astype(bf16), u32)
                    kv_v[pl.ds((g * RG + c * RC) // 2, RC // 2), _tile(j)] = b
                    lhs.append(b)
            res = _dot(_unpack(jnp.concatenate(lhs, axis=0)), ft_v[...])
            for c in range(NRC):
                for j in range(Q):
                    sp_v[g][self.ub + j, pl.ds(c * RC, RC), :] = piece(res, c, j)

        def chain(self, g, p, init, terms):
            pu, ph = pl.ds(p * 8, 8), pl.ds(p * 8 + HOFF, 8)
            link = lambda a, i: a if self.first else jnp.where(self.keep, a, self.prev[i])
            ar, ai = (None, None) if init is None else (link(init[0], 0), link(init[1], 1))
            for j, m in terms:
                ur, ui = sp_v[g][j, pu, :BK], sp_v[g][j, pu, BK:]
                hr, hi = sp_v[g][m, ph, :BK], sp_v[g][m, ph, BK:]
                if ar is None:
                    ar, ai = link(ur * hr, 0) - ui * hi, link(ur * hi, 1) + ui * hr
                elif self.first:
                    ar, ai = ar + (ur * hr - ui * hi), ai + (ur * hi + ui * hr)
                else:
                    ar, ai = (ar + ur * hr) - ui * hi, (ai + ur * hi) + ui * hr
            self.prev = (ar, ai)
            return ar, ai

        def mac(self, p0, p1):
            for pp in range(p0, p1):
                g, p = divmod(pp, PG)
                pr = pl.ds(p * 8, 8)
                for a in range(Q):
                    terms = [(self.ub + b, HL + a - b) for b in range(a + 1)]
                    init = None
                    if not self.first:
                        init = (part_v[g][a, pr, :BK], part_v[g][a, pr, BK:])
                        terms = [(U0 + b, HW + Q - 1 + a - b) for b in range(Q)] + terms
                    yf_v[g][a, pr, :BK], yf_v[g][a, pr, BK:] = self.chain(g, p, init, terms)

        def mac_ahead(self, p0, p1):
            for pp in range(p0, p1):
                g, p = divmod(pp, PG)
                pr = pl.ds(p * 8, 8)
                for a in range(Q):
                    terms = ([(UP + b, HW + Q - 1 + a - b) for b in range(Q)]
                             + [(UC + b, HL + Q + a - b) for b in range(Q)])
                    part_v[g][a, pr, :BK], part_v[g][a, pr, BK:] = self.chain(g, p, None, terms)
                ph = pl.ds(p * 8 + HOFF, 8)
                moves = [(UP + b, UC + b, pr) for b in range(Q)] + [(HW + b, HW + Q + b, ph) for b in range(Q - 1)]
                for dst, src, rows in moves:
                    for i in range(2):
                        sp_v[g][dst, rows, _tile(i)] = jnp.where(self.keep, sp_v[g][src, rows, _tile(i)], self.prev[i])

    def inv_tile(t):
        halves = [_dot(jnp.concatenate([yf_v[g][t] for g in (2 * hh, 2 * hh + 1)], axis=0).astype(bf16), gt_v[...])
                  for hh in range(2)]
        return jnp.concatenate(halves, axis=0) + _unpack(kv_v[:, _tile(t)]).astype(f32) * col_v[4]

    def inv_group(g):
        rows = slice(g * RG, (g + 1) * RG)
        res = _dot(jnp.concatenate([yf_v[g][j] for j in range(Q)], axis=0).astype(bf16), gt_v[...])
        kv = _unpack(kv_v[g * RG // 2:(g + 1) * RG // 2, :]).astype(f32)
        for j in range(Q):
            y_v[rows, _tile(j)] = res[j * RG:(j + 1) * RG] + kv[:, _tile(j)] * col_v[4, rows, :]

    def stage(x, y):
        x = x + _ln(x) * y
        return x, _ln(x).astype(bf16)

    def mm1(xn):
        return _silu(_dot(_unpack(w1p_v[...]), xn))

    def cut(g):
        return [g[a * BK:b * BK].astype(bf16) for a, b in zip(KS[:-1], KS[1:])]

    def head2(w, g0):
        return jnp.concatenate([_dot(w[:D // 2], g0), _dot(w[D // 2:], g0)], axis=0)

    def mm2(x, gs):
        w = _unpack(w2p_v[...])
        k0, k1 = KS[1] * BK, KS[2] * BK
        mid = head2(w[:, :k0], gs[0]) + _dot(w[:, k0:k1], gs[1])
        return x + (mid + _dot(w[:, k1:], gs[2])), mid[D - 8:]

    cv = Conv(0)
    for c in c_taps: c.wait()
    sh = sh_v[...].astype(f32)
    dd = d_v[...].astype(f32).reshape(1, D)
    for t in range(5):
        col_v[t] = jnp.broadcast_to(sh[t:t + 1, :] if t < 4 else dd, (BK, D)).T
    for c in c_h0: c.wait()
    for c in [c_gt] + c_kv1 + [c_q0]: c.start()
    for g in range(NG): cv.fwd_h(g)
    for c in c_kv0: c.wait()
    for c in range(3): w1_copy(c).start()
    cv.fwd_u(0); cv.fwd_u(1)
    c_gt.wait()
    cv.mac(0, 2 * PG)
    inv_group(0); inv_group(1)
    for c in c_kv1: c.wait()
    w1_copy(3).start()
    cv.fwd_u(2); cv.fwd_u(3)

    def transpose_w1(c):
        w1p_v[W1B[c] // 2:W1B[c + 1] // 2, :] = pltpu.bitcast(w1_v[:, W1B[c]:W1B[c + 1]].T, u32)

    xs, xns, gs = [None] * Q, [None] * Q, [[] for _ in range(Q)]

    def mm1_part(c, t):
        g = _silu(_dot(_unpack(w1p_v[W1B[c] // 2:W1B[c + 1] // 2, :]), xns[t]))
        gs[t].append(g.astype(bf16))
        return g

    c_q0.wait()
    w1_copy(0).wait()
    c_w2.start()
    cv.mac(2 * PG, NP)
    inv_group(2); inv_group(3)
    transpose_w1(0)
    xs[0], xns[0] = stage(q_v[:, _tile(0)].astype(f32), y_v[:, _tile(0)])
    w1_copy(1).wait(); w1_copy(2).wait()
    transpose_w1(1); transpose_w1(2)
    keep = all_true()
    for t in range(Q):
        for c in range(3 if t < Q - 1 else 2):
            g = mm1_part(c, t)
            if c == 0 and t + 1 < Q:
                x = tie(q_v[:, _tile(t + 1)].astype(f32), keep, g[0:8])
                xs[t + 1], xns[t + 1] = stage(x, y_v[:, _tile(t + 1)])
    w1_copy(3).wait()
    transpose_w1(3)
    keep = all_true()
    mm1_part(2, Q - 1)
    paced = []
    for t in range(Q - 1):
        g = mm1_part(3, t)
        paced += [g[i * 8:(i + 1) * 8] for i in range(0, 96, 9)]
    for i in range(2 * NG * Q):
        z = jnp.tile(jnp.where(keep, 0.0, paced[i]), (PG, 2))
        g, a = divmod(i % (NG * Q), Q)
        if i < NG * Q:
            part_v[g][a] = z
        else:
            sp_v[g][UP + a, :RG] = z
    c_w2.wait()
    for c in step_copies(1): c.start()
    mm1_part(3, Q - 1)
    for c in range(W1C):
        gc_v[W1B[c] // 2:W1B[c + 1] // 2, :] = pltpu.bitcast(gs[Q - 1][c], u32)
    x1_v[...] = xs[Q - 1]
    w2t = w2t_v[...]
    w2p_v[...] = pltpu.bitcast(w2t, u32)
    for t in range(Q - 1):
        acc = head2(w2t[:, :W1B[1]], gs[t][0])
        for c in range(1, W1C):
            acc = acc + _dot(w2t[:, W1B[c]:W1B[c + 1]], gs[t][c])
        x2_v[:, _tile(t)] = xs[t] + acc

    def step(s, carry):
        for c in step_copies(s + 1): c.wait()

        @pl.when(s + 2 < NS)
        def _():
            for c in step_copies(s + 2): c.start()

        cv = Conv(s + 1)
        o0 = pl.multiple_of(s * T, T)
        q0 = pl.multiple_of((s + 1) * T, T)

        w2, gc = _unpack(w2p_v[...]), _unpack(gc_v[...])
        part = lambda a, b: (w2[:, a * BK:b * BK], gc[a * BK:b * BK])
        cv.fwd_h(0); acc = x1_v[...] + _dot(*part(0, 2))
        cv.fwd_u(0); cv.fwd_h(1)
        cv.fwd_u(1); cv.fwd_h(2)
        cv.fwd_u(2); cv.fwd_h(3)
        cv.fwd_u(3); acc = acc + _dot(*part(2, 4))
        hd = head2(*part(4, 6))
        x2_v[:, _tile(Q - 1)] = acc + hd + _dot(*part(6, F // BK))
        x, xn = stage(x2_v[:, _tile(0)], tie(y_v[:, _tile(0)], cv.keep, hd[D - 8:]))
        split()

        for t in range(Q):
            g = mm1(xn)
            if t == 0:
                cv.anchor(g[0:8]); cv.mac(CB[0], CB[1])
            if t == Q - 1:
                cv.keep = all_true()
                y = inv_tile(0)
            o, mid = mm2(x, cut(g))
            o_v[:, pl.ds(o0 + t * BK, BK)] = o.astype(bf16)
            cv.anchor(mid)
            if t < Q - 1:
                x, xn = stage(tie(x2_v[:, _tile(t + 1)], cv.keep, g[F - 8:]), y_v[:, _tile(t + 1)])
                cv.mac(CB[t + 1], CB[t + 2])
                if t == Q - 2:
                    cv.mac_ahead(BB[0], BB[1])
        for t in range(Q):
            x, xn = stage(q_v[:, pl.ds(q0 + t * BK, BK)].astype(f32), y)
            y_v[:, _tile(t)] = y
            cv.mac_ahead(BB[t + 1], BB[t + 2])
            g = mm1(xn)
            if t + 1 < Q:
                y = inv_tile(t + 1)
                x2_v[:, _tile(t)], mid = mm2(x, cut(g))
                cv.anchor(mid)
            else:
                gc_v[...] = pltpu.bitcast(g.astype(bf16), u32)
                x1_v[...] = x
        out_copy(o0, T).start()
        return carry

    lax.fori_loop(0, NS - 1, step, 0)

    gc = _unpack(gc_v[...])
    x2_v[:, _tile(Q - 1)] = mm2(x1_v[...], [gc[a * BK:b * BK] for a, b in zip(KS[:-1], KS[1:])])[0]
    for t in range(Q):
        x, xn = stage(x2_v[:, _tile(t)], y_v[:, _tile(t)])
        c0 = (NS - 1) * T + t * BK
        o_v[:, c0:c0 + BK] = mm2(x, cut(mm1(xn)))[0].astype(bf16)
        out_copy(c0, BK).start()
    out_copy(0, S).wait()


@jax.jit
def pallas_interleave_layers__ssm_conv_h3__dense_activation_silu__prompt_kernel(
        A_q, A_k, A_v, A_shift_k, A_ssm_k, A_ssm_D, B_x, B_w1, B_w2):
    ft, gt = _tables()
    act = pltpu.VMEM((D, S), bf16)
    wgt = pltpu.VMEM((D, F), bf16)
    groups = ([pltpu.VMEM((NSP, RG + 2 * HOFF, 2 * BK), f32)] * NG + [pltpu.VMEM((RG, 2 * BK), f32)] * NG
              + [pltpu.VMEM((Q, RG, 2 * BK), f32)] * (2 * NG))
    out = pl.pallas_call(
        _kernel,
        in_specs=[pl.BlockSpec(memory_space=pl.ANY)] * 10,
        out_specs=pl.BlockSpec(memory_space=pl.ANY),
        out_shape=jax.ShapeDtypeStruct((D, S), bf16),
        scratch_shapes=[act] * 5 + [
            pltpu.VMEM((4, D), bf16), pltpu.VMEM((D,), bf16), wgt, wgt,
            pltpu.VMEM((F // 2, D), u32), pltpu.VMEM((D // 2, F), u32),
            pltpu.VMEM((BK, 2 * BK), bf16), pltpu.VMEM((2 * BK, BK), bf16),
            pltpu.VMEM((5, D, BK), f32), pltpu.VMEM((8, BK), i32), pltpu.SMEM((1,), i32),
            pltpu.VMEM((D // 2, T), u32), pltpu.VMEM((D, T), f32), pltpu.VMEM((D, T), f32),
            pltpu.VMEM((F // 2, BK), u32), pltpu.VMEM((D, BK), f32),
            pltpu.SemaphoreType.DMA((7,)), pltpu.SemaphoreType.DMA((W1C,)),
            pltpu.SemaphoreType.DMA((NS - 1,)), pltpu.SemaphoreType.DMA] + groups,
        compiler_params=pltpu.CompilerParams(vmem_limit_bytes=110 * 1024 * 1024, disable_bounds_checks=True,
                                             disable_semaphore_checks=True),
    )(A_q.reshape(S, D).T, A_k.reshape(S, D).T, A_v.reshape(S, D).T, A_shift_k.T, A_ssm_k, A_ssm_D,
      B_w1, B_w2.T, ft, gt)
    return out.T.reshape(1, S, D)
```

```python
import jax
import jax.numpy as jnp
import numpy as np
from jax import lax
import jax.experimental.pallas as pl
import jax.experimental.pallas.tpu as pltpu

S, D, F = 2048, 448, 1792
BK = 128
NB = S // BK
T = 512
Q = T // BK
NS = S // T
RG = 112
NG = D // RG
PG = RG // 8
NP = NG * PG
RC = 16
NRC = RG // RC
W1B = (0, 256, 512, 1024, 1792)
W1C = len(W1B) - 1
U0, UC, UP, HL, HW, NSP = 0, 4, 8, 12, 24, 31
HOFF = 8
CB = (0, 19, 38, 56)
BB = (0, 2, 5, 9, 20, 32, 44, 56)
EPS = 1e-5
f32, bf16, u32, i32 = jnp.float32, jnp.bfloat16, jnp.uint32, jnp.int32


def _dft_table(shape, n_axis, scale):
    n = lax.broadcasted_iota(i32, shape, n_axis)
    kk = lax.broadcasted_iota(i32, shape, 1 - n_axis)
    ph = (4 * (kk & (BK - 1)) + 1) * n - (kk & BK)
    phi = ((ph & (2 * BK - 1)) - BK).astype(f32) * (np.pi / (2 * BK))
    p2 = phi * phi
    s = 1.0 / 39916800
    for d in (362880, 5040, 120, 6, 1):
        s = 1.0 / d - p2 * s
    s = s * phi
    return (jnp.where((ph & (2 * BK)) == 0, -scale, scale) * s).astype(bf16)


def _ln(x):
    m = jnp.sum(x, axis=0, keepdims=True) * (1.0 / D)
    xc = x - m
    v = jnp.sum(xc * xc, axis=0, keepdims=True) * (1.0 / D)
    return xc * lax.rsqrt(v + EPS)


def _silu(h):
    t = 0.5 * h
    return t * jnp.tanh(t) + t


def _dot(a, b):
    return jnp.dot(a, b, preferred_element_type=f32)


def _unpack(x):
    return pltpu.bitcast(x, bf16)


def _tile(t):
    return slice(t * BK, (t + 1) * BK)


def _kernel(q_hbm, k_hbm, v_hbm, sh_hbm, h_hbm, d_hbm, w1_hbm, w2t_hbm, o_hbm,
            q_v, k_v, v_v, h_v, o_v, sh_v, d_v, w1_v, w2t_v, w1p_v, w2p_v, ft_v, gt_v, col_v, zero_v,
            kv_v, y_v, x2_v, gc_v, x1_v, sem, wsem, osem, *grp):
    sp_v, hraw_v, part_v, yf_v = (grp[i * NG:(i + 1) * NG] for i in range(4))

    def step_copy(src, dst, s, sm, halo=0):
        return pltpu.make_async_copy(src.at[:, pl.ds(pl.multiple_of(s * T - halo, BK), T + halo)], dst, sm)

    def conv_copies(s):
        return [step_copy(k_hbm, k_v, s, sem.at[6], BK), step_copy(v_hbm, v_v, s, sem.at[6]),
                step_copy(h_hbm, h_v, s, sem.at[6])]

    def half_copies(hh, sk, sv):
        rows = pl.ds(hh * 2 * RG, 2 * RG)
        return [pltpu.make_async_copy(k_hbm.at[rows, pl.ds(0, T)], k_v.at[rows, pl.ds(BK, T)], sk),
                pltpu.make_async_copy(v_hbm.at[rows, pl.ds(0, T)], v_v.at[rows], sv)]

    def w1_copy(c):
        cols = pl.ds(W1B[c], W1B[c + 1] - W1B[c])
        return pltpu.make_async_copy(w1_hbm.at[:, cols], w1_v.at[:, cols], wsem.at[c])

    def out_copy(c0, w):
        cols = pl.ds(c0, w)
        return pltpu.make_async_copy(o_v.at[:, cols], o_hbm.at[:, cols], osem)

    c_taps = [pltpu.make_async_copy(sh_hbm, sh_v, sem.at[0]), pltpu.make_async_copy(d_hbm, d_v, sem.at[0])]
    c_h0 = [step_copy(h_hbm, h_v, 0, sem.at[1])]
    c_kv0 = half_copies(0, sem.at[2], sem.at[2])
    c_kv1 = half_copies(1, sem.at[7], sem.at[3])
    c_q0 = step_copy(q_hbm, q_v, 0, sem.at[4])
    c_w2 = pltpu.make_async_copy(w2t_hbm, w2t_v, sem.at[5])
    for c in c_taps + c_h0 + c_kv0:
        c.start()
    zero_v[...] = jnp.zeros(zero_v.shape, i32)
    ft_v[...] = pltpu.bitcast(_dft_table((BK, 2 * BK), 0, 1.0), u32)
    gt_v[...] = pltpu.bitcast(_dft_table((2 * BK, BK), 1, 1.0 / BK), u32)

    def all_true():
        return zero_v[...] == 0

    def tie(val, keep, dep):
        return jnp.concatenate([jnp.where(keep, val[0:8], dep), val[8:]], axis=0)

    def piece(res, c, j):
        return res[(c * Q + j) * RC:(c * Q + j + 1) * RC]

    class Conv:
        def __init__(self, q):
            self.q = q
            self.first = isinstance(q, int)
            self.ub = U0 if self.first else UC
            self.keep = None if self.first else all_true()
            self.prev = None

        def anchor(self, val):
            self.prev = (val, val)

        def fwd_h(self, g):
            hh = h_v[pl.ds(g * RG, RG), :]
            lhs = jnp.concatenate([hh[c * RC:(c + 1) * RC, _tile(j)] for c in range(NRC) for j in range(Q)], axis=0)
            res = _dot(lhs, _unpack(ft_v[...]))
            low = HL + Q * jnp.minimum(self.q, 2)
            for c in range(NRC):
                r = pl.ds(c * RC, RC)
                rh = pl.ds(c * RC + HOFF, RC)
                for j in range(Q):
                    hp = piece(res, c, j)
                    if j > 0 or not self.first:
                        prev = hraw_v[g][r, :] if j == 0 else piece(res, c, j - 1)
                        hp = jnp.concatenate([hp[:, :BK] + prev[:, BK:], hp[:, BK:] - prev[:, :BK]], axis=1)
                    if self.first:
                        sp_v[g][HL + j, rh, :] = hp
                        if j > 0:
                            sp_v[g][HW + j - 1, rh, :] = hp
                    else:
                        sp_v[g][HW + Q - 1 + j, rh, :] = hp
                        sp_v[g][low + j, rh, :] = hp
                hraw_v[g][r, :] = piece(res, c, Q - 1)

        def fwd_u(self, g):
            lhs = []
            for c in range(NRC):
                r = pl.ds(g * RG + c * RC, RC)
                if self.first:
                    kk = jnp.concatenate([jnp.zeros((RC // 2, BK), u32), pltpu.bitcast(k_v[r, BK:], u32)], axis=1)
                else:
                    kk = pltpu.bitcast(k_v[r, :], u32)
                ks = None
                for tau in range(4):
                    shifted = kk if tau == 0 else pltpu.roll(kk, tau, 1)
                    term = _unpack(shifted[:, BK:]).astype(f32) * jnp.tile(col_v[tau, r, :], (1, Q))
                    ks = term if ks is None else ks + term
                kv = ks * v_v[r, :].astype(f32)
                for j in range(Q):
                    b = pltpu.bitcast(kv[:, _tile(j)].astype(bf16), u32)
                    kv_v[pl.ds((g * RG + c * RC) // 2, RC // 2), _tile(j)] = b
                    lhs.append(b)
            res = _dot(_unpack(jnp.concatenate(lhs, axis=0)), _unpack(ft_v[...]))
            for c in range(NRC):
                for j in range(Q):
                    sp_v[g][self.ub + j, pl.ds(c * RC, RC), :] = piece(res, c, j)

        def chain(self, g, p, init, terms):
            pu, ph = pl.ds(p * 8, 8), pl.ds(p * 8 + HOFF, 8)
            link = lambda a, i: a if self.first else jnp.where(self.keep, a, self.prev[i])
            ar, ai = (None, None) if init is None else (link(init[0], 0), link(init[1], 1))
            for j, m in terms:
                ur, ui = sp_v[g][j, pu, :BK], sp_v[g][j, pu, BK:]
                hr, hi = sp_v[g][m, ph, :BK], sp_v[g][m, ph, BK:]
                if ar is None:
                    ar, ai = link(ur * hr, 0) - ui * hi, link(ur * hi, 1) + ui * hr
                elif self.first:
                    ar, ai = ar + (ur * hr - ui * hi), ai + (ur * hi + ui * hr)
                else:
                    ar, ai = (ar + ur * hr) - ui * hi, (ai + ur * hi) + ui * hr
            self.prev = (ar, ai)
            return ar, ai

        def mac(self, p0, p1):
            for pp in range(p0, p1):
                g, p = divmod(pp, PG)
                pr = pl.ds(p * 8, 8)
                for a in range(Q):
                    terms = [(self.ub + b, HL + a - b) for b in range(a + 1)]
                    init = None
                    if not self.first:
                        init = (part_v[g][a, pr, :BK], part_v[g][a, pr, BK:])
                        terms = [(U0 + b, HW + Q - 1 + a - b) for b in range(Q)] + terms
                    yf_v[g][a, pr, :BK], yf_v[g][a, pr, BK:] = self.chain(g, p, init, terms)

        def mac_ahead(self, p0, p1):
            for pp in range(p0, p1):
                g, p = divmod(pp, PG)
                pr = pl.ds(p * 8, 8)
                for a in range(Q):
                    terms = ([(UP + b, HW + Q - 1 + a - b) for b in range(Q)]
                             + [(UC + b, HL + Q + a - b) for b in range(Q)])
                    part_v[g][a, pr, :BK], part_v[g][a, pr, BK:] = self.chain(g, p, None, terms)
                ph = pl.ds(p * 8 + HOFF, 8)
                moves = [(UP + b, UC + b, pr) for b in range(Q)] + [(HW + b, HW + Q + b, ph) for b in range(Q - 1)]
                for dst, src, rows in moves:
                    for i in range(2):
                        sp_v[g][dst, rows, _tile(i)] = jnp.where(self.keep, sp_v[g][src, rows, _tile(i)], self.prev[i])

    def inv_tile(t):
        halves = [_dot(jnp.concatenate([yf_v[g][t] for g in (2 * hh, 2 * hh + 1)], axis=0).astype(bf16), _unpack(gt_v[...]))
                  for hh in range(2)]
        return jnp.concatenate(halves, axis=0) + _unpack(kv_v[:, _tile(t)]).astype(f32) * col_v[4]

    def inv_group(g):
        rows = slice(g * RG, (g + 1) * RG)
        res = _dot(jnp.concatenate([yf_v[g][j] for j in range(Q)], axis=0).astype(bf16), _unpack(gt_v[...]))
        kv = _unpack(kv_v[g * RG // 2:(g + 1) * RG // 2, :]).astype(f32)
        for j in range(Q):
            y_v[rows, _tile(j)] = res[j * RG:(j + 1) * RG] + kv[:, _tile(j)] * col_v[4, rows, :]

    def stage(x, y):
        x = x + _ln(x) * y
        return x, _ln(x).astype(bf16)

    def mm1(xn):
        return _silu(_dot(_unpack(w1p_v[...]), xn))

    def head2(w, g0):
        return jnp.concatenate([_dot(w[:D // 2], g0), _dot(w[D // 2:], g0)], axis=0)

    def mm2(x, g):
        w, k0 = _unpack(w2p_v[...]), 2 * BK
        return x + (head2(w[:, :k0], g[:k0].astype(bf16)) + _dot(w[:, k0:], g[k0:].astype(bf16)))

    cv = Conv(0)
    for c in c_taps: c.wait()
    sh = sh_v[...].astype(f32)
    dd = d_v[...].astype(f32).reshape(1, D)
    for t in range(5):
        col_v[t] = jnp.broadcast_to(sh[t:t + 1, :] if t < 4 else dd, (BK, D)).T
    for c in c_h0: c.wait()
    for c in c_kv1 + [c_q0]: c.start()
    for g in range(NG): cv.fwd_h(g)
    for c in c_kv0: c.wait()
    for c in range(3): w1_copy(c).start()
    cv.fwd_u(0); cv.fwd_u(1)
    c_kv1[0].wait()
    cv.mac(0, 2 * PG)
    inv_group(0); inv_group(1)
    c_kv1[1].wait()
    w1_copy(3).start()
    cv.fwd_u(2); cv.fwd_u(3)

    def transpose_w1(c):
        w1p_v[W1B[c] // 2:W1B[c + 1] // 2, :] = pltpu.bitcast(w1_v[:, W1B[c]:W1B[c + 1]].T, u32)

    xs, xns, gs = [None] * Q, [None] * Q, [[] for _ in range(Q)]

    def mm1_part(c, t):
        g = _silu(_dot(_unpack(w1p_v[W1B[c] // 2:W1B[c + 1] // 2, :]), xns[t]))
        gs[t].append(g.astype(bf16))
        return g

    c_q0.wait()
    w1_copy(0).wait()
    c_w2.start()
    cv.mac(2 * PG, NP)
    inv_group(2); inv_group(3)
    transpose_w1(0)
    xs[0], xns[0] = stage(q_v[:, _tile(0)].astype(f32), y_v[:, _tile(0)])
    w1_copy(1).wait(); w1_copy(2).wait()
    transpose_w1(1); transpose_w1(2)
    keep = all_true()
    for t in range(Q):
        for c in range(3 if t < Q - 1 else 2):
            g = mm1_part(c, t)
            if c == 0 and t + 1 < Q:
                x = tie(q_v[:, _tile(t + 1)].astype(f32), keep, g[0:8])
                xs[t + 1], xns[t + 1] = stage(x, y_v[:, _tile(t + 1)])
    w1_copy(3).wait()
    transpose_w1(3)
    keep = all_true()
    mm1_part(2, Q - 1)
    paced = []
    for t in range(Q - 1):
        g = mm1_part(3, t)
        paced += [g[i * 8:(i + 1) * 8] for i in range(0, 96, 9)]
    for i in range(2 * NG * Q):
        z = jnp.tile(jnp.where(keep, 0.0, paced[i]), (PG, 2))
        g, a = divmod(i % (NG * Q), Q)
        if i < NG * Q:
            part_v[g][a] = z
        else:
            sp_v[g][UP + a, :RG] = z
    c_w2.wait()
    for c in conv_copies(1): c.start()
    mm1_part(3, Q - 1)
    for c in range(W1C):
        gc_v[W1B[c] // 2:W1B[c + 1] // 2, :] = pltpu.bitcast(gs[Q - 1][c], u32)
    x1_v[...] = xs[Q - 1]
    w2t = w2t_v[...]
    w2p_v[...] = pltpu.bitcast(w2t, u32)
    for t in range(Q - 1):
        acc = head2(w2t[:, :W1B[1]], gs[t][0])
        for c in range(1, W1C):
            acc = acc + _dot(w2t[:, W1B[c]:W1B[c + 1]], gs[t][c])
        x2_v[:, _tile(t)] = xs[t] + acc

    def step(s, carry):
        for c in conv_copies(s + 1): c.wait()
        c_q = step_copy(q_hbm, q_v, s + 1, sem.at[4])
        c_q.start()
        cv = Conv(s + 1)
        o0 = pl.multiple_of(s * T, T)

        w2, gc = _unpack(w2p_v[...]), _unpack(gc_v[...])
        part = lambda a, b: (w2[:, a * BK:b * BK], gc[a * BK:b * BK])
        cv.fwd_h(0); acc = x1_v[...] + _dot(*part(0, 2))
        cv.fwd_u(0); cv.fwd_h(1)
        cv.fwd_u(1); cv.fwd_h(2)
        cv.fwd_u(2); cv.fwd_h(3)
        cv.fwd_u(3); acc = acc + _dot(*part(2, 4))
        hd = head2(*part(4, 6))
        x2_v[:, _tile(Q - 1)] = acc + hd + _dot(*part(6, F // BK))
        x, xn = stage(x2_v[:, _tile(0)], tie(y_v[:, _tile(0)], cv.keep, hd[D - 8:]))
        c_q.wait()

        @pl.when(s + 2 < NS)
        def _():
            for c in conv_copies(s + 2): c.start()

        for t in range(Q):
            g = mm1(xn)
            cv.anchor(g[0:8])
            if t < Q - 1:
                cv.mac(CB[t], CB[t + 1])
            cv.mac_ahead(BB[t], BB[t + 1])
            if t == Q - 1:
                y = inv_tile(0)
            o_v[:, pl.ds(o0 + t * BK, BK)] = mm2(x, g).astype(bf16)
            if t < Q - 1:
                x, xn = stage(x2_v[:, _tile(t + 1)], y_v[:, _tile(t + 1)])
        for t in range(Q):
            x, xn = stage(q_v[:, _tile(t)].astype(f32), y)
            y_v[:, _tile(t)] = y
            g = mm1(xn)
            if t + 1 < Q:
                cv.anchor(g[0:8])
                cv.mac_ahead(BB[Q + t], BB[Q + t + 1])
                y = inv_tile(t + 1)
                x2_v[:, _tile(t)] = mm2(x, g)
            else:
                gc_v[...] = pltpu.bitcast(g.astype(bf16), u32)
                x1_v[...] = x
        out_copy(o0, T).start()
        return carry

    lax.fori_loop(0, NS - 1, step, 0)

    x2_v[:, _tile(Q - 1)] = mm2(x1_v[...], _unpack(gc_v[...]))
    for t in range(Q):
        x, xn = stage(x2_v[:, _tile(t)], y_v[:, _tile(t)])
        c0 = (NS - 1) * T + t * BK
        o_v[:, c0:c0 + BK] = mm2(x, mm1(xn)).astype(bf16)
        out_copy(c0, BK).start()
    out_copy(0, S).wait()


@jax.jit
def pallas_interleave_layers__ssm_conv_h3__dense_activation_silu__prompt_kernel(
        A_q, A_k, A_v, A_shift_k, A_ssm_k, A_ssm_D, B_x, B_w1, B_w2):
    act = pltpu.VMEM((D, T), bf16)
    wgt = pltpu.VMEM((D, F), bf16)
    groups = ([pltpu.VMEM((NSP, RG + 2 * HOFF, 2 * BK), f32)] * NG + [pltpu.VMEM((RG, 2 * BK), f32)] * NG
              + [pltpu.VMEM((Q, RG, 2 * BK), f32)] * (2 * NG))
    out = pl.pallas_call(
        _kernel,
        in_specs=[pl.BlockSpec(memory_space=pl.ANY)] * 8,
        out_specs=pl.BlockSpec(memory_space=pl.ANY),
        out_shape=jax.ShapeDtypeStruct((D, S), bf16),
        scratch_shapes=[act, pltpu.VMEM((D, T + BK), bf16), act, act, pltpu.VMEM((D, S), bf16)] + [
            pltpu.VMEM((4, D), bf16), pltpu.VMEM((D,), bf16), wgt, wgt,
            pltpu.VMEM((F // 2, D), u32), pltpu.VMEM((D // 2, F), u32),
            pltpu.VMEM((BK // 2, 2 * BK), u32), pltpu.VMEM((BK, BK), u32),
            pltpu.VMEM((5, D, BK), f32), pltpu.VMEM((8, BK), i32),
            pltpu.VMEM((D // 2, T), u32), pltpu.VMEM((D, T), f32), pltpu.VMEM((D, T), f32),
            pltpu.VMEM((F // 2, BK), u32), pltpu.VMEM((D, BK), f32),
            pltpu.SemaphoreType.DMA((8,)), pltpu.SemaphoreType.DMA((W1C,)), pltpu.SemaphoreType.DMA] + groups,
        compiler_params=pltpu.CompilerParams(vmem_limit_bytes=110 * 1024 * 1024, disable_bounds_checks=True,
                                             disable_semaphore_checks=True),
    )(A_q.reshape(S, D).T, A_k.reshape(S, D).T, A_v.reshape(S, D).T, A_shift_k.T, A_ssm_k, A_ssm_D,
      B_w1, B_w2.T)
    return out.T.reshape(1, S, D)
```

```python
import jax
import jax.numpy as jnp
import numpy as np
from jax import lax
import jax.experimental.pallas as pl
import jax.experimental.pallas.tpu as pltpu

S, D, F = 2048, 448, 1792
BK = 128
T = 512
Q = T // BK
NS = S // T
RG = 112
NG = D // RG
PG = RG // 8
NP = NG * PG
RC = 16
NRC = RG // RC
W1B = (0, 256, 512, 1024, 1792)
W1C = len(W1B) - 1
U0, UC, UP, HL, HW, NSP = 0, 4, 8, 12, 24, 31
HOFF = 8
CB = (0, 19, 38, 56)
BB = (0, 2, 5, 9, 20, 32, 44, 56)
EPS = 1e-5
LAST = ((0, 208), (208, 416), (416, 448))
f32, bf16, u32, i32 = jnp.float32, jnp.bfloat16, jnp.uint32, jnp.int32


def _dft_table(shape, n_axis, scale):
    n = lax.broadcasted_iota(i32, shape, n_axis)
    kk = lax.broadcasted_iota(i32, shape, 1 - n_axis)
    ph = (4 * (kk & (BK - 1)) + 1) * n - (kk & BK)
    phi = ((ph & (2 * BK - 1)) - BK).astype(f32) * (np.pi / (2 * BK))
    p2 = phi * phi
    s = 1.0 / 39916800
    for d in (362880, 5040, 120, 6, 1):
        s = 1.0 / d - p2 * s
    s = s * phi
    return (jnp.where((ph & (2 * BK)) == 0, -scale, scale) * s).astype(bf16)


def _ln(x):
    m = jnp.sum(x, axis=0, keepdims=True) * (1.0 / D)
    xc = x - m
    v = jnp.sum(xc * xc, axis=0, keepdims=True) * (1.0 / D)
    return xc * lax.rsqrt(v + EPS)


def _silu(h):
    t = 0.5 * h
    return t * jnp.tanh(t) + t


def _dot(a, b):
    return jnp.dot(a, b, preferred_element_type=f32)


def _unpack(x):
    return pltpu.bitcast(x, bf16)


def _halves(z):
    return z[:, :BK], z[:, BK:]


def _tile(t):
    return slice(t * BK, (t + 1) * BK)


def _kernel(q_hbm, k_hbm, v_hbm, sh_hbm, h_hbm, d_hbm, w1_hbm, w2t_hbm, o_hbm,
            q_v, k_v, v_v, h_v, o_v, sh_v, d_v, w1_v, w2t_v, w1p_v, w2p_v, ft_v, gt_v, col_v, zero_v,
            kv_v, y_v, x2_v, gc_v, x1_v, sem, wsem, osem, *grp):
    sp_v, hraw_v, part_v, yf_v = (grp[i * NG:(i + 1) * NG] for i in range(4))

    def step_copy(src, dst, s, sm, halo=0):
        return pltpu.make_async_copy(src.at[:, pl.ds(pl.multiple_of(s * T - halo, BK), T + halo)], dst, sm)

    def conv_copies(s):
        return [step_copy(k_hbm, k_v, s, sem.at[6], BK), step_copy(v_hbm, v_v, s, sem.at[6]),
                step_copy(h_hbm, h_v, s, sem.at[6])]

    def half_copies(hh, sk, sv):
        rows = pl.ds(hh * 2 * RG, 2 * RG)
        return [pltpu.make_async_copy(k_hbm.at[rows, pl.ds(0, T)], k_v.at[rows, pl.ds(BK, T)], sk),
                pltpu.make_async_copy(v_hbm.at[rows, pl.ds(0, T)], v_v.at[rows], sv)]

    def w1_copy(c):
        cols = pl.ds(W1B[c], W1B[c + 1] - W1B[c])
        return pltpu.make_async_copy(w1_hbm.at[:, cols], w1_v.at[:, cols], wsem.at[c])

    def out_copy(c0, w):
        cols = pl.ds(c0, w)
        return pltpu.make_async_copy(o_v.at[:, cols], o_hbm.at[:, cols], osem)

    c_taps = [pltpu.make_async_copy(sh_hbm, sh_v, sem.at[0]), pltpu.make_async_copy(d_hbm, d_v, sem.at[0])]
    c_h0 = [step_copy(h_hbm, h_v, 0, sem.at[1])]
    c_kv0 = half_copies(0, sem.at[2], sem.at[2])
    c_kv1 = half_copies(1, sem.at[7], sem.at[3])
    c_q0 = step_copy(q_hbm, q_v, 0, sem.at[4])
    c_w2 = pltpu.make_async_copy(w2t_hbm, w2t_v, sem.at[5])
    for c in c_taps + c_h0 + c_kv0:
        c.start()
    zero_v[...] = jnp.zeros(zero_v.shape, i32)
    ft_v[...] = pltpu.bitcast(_dft_table((BK, 2 * BK), 0, 1.0), u32)
    gt_v[...] = pltpu.bitcast(_dft_table((2 * BK, BK), 1, 1.0 / BK), u32)

    def all_true():
        return zero_v[...] == 0

    def tie(val, keep, dep):
        return jnp.concatenate([lax.select(keep, val[0:8], dep), val[8:]], axis=0)

    def piece(res, c, j):
        return res[(c * Q + j) * RC:(c * Q + j + 1) * RC]

    class Conv:
        def __init__(self, q):
            self.q = q
            self.first = isinstance(q, int)
            self.ub = U0 if self.first else UC
            self.keep = None if self.first else all_true()
            self.low = None if self.first else HL + Q * jnp.minimum(q, 2)
            self.prev = None

        def anchor(self, val):
            self.prev = (val, val)

        def fwd_h(self, g):
            hh = h_v[pl.ds(g * RG, RG), :]
            lhs = jnp.concatenate([hh[c * RC:(c + 1) * RC, _tile(j)] for c in range(NRC) for j in range(Q)], axis=0)
            res = _dot(lhs, _unpack(ft_v[...]))
            for c in range(NRC):
                r = pl.ds(c * RC, RC)
                rh = pl.ds(c * RC + HOFF, RC)
                for j in range(Q):
                    hp = piece(res, c, j)
                    if j > 0 or not self.first:
                        prev = hraw_v[g][r, :] if j == 0 else piece(res, c, j - 1)
                        hp = jnp.concatenate([hp[:, :BK] + prev[:, BK:], hp[:, BK:] - prev[:, :BK]], axis=1)
                    if self.first:
                        sp_v[g][HL + j, rh, :] = hp
                        if j > 0:
                            sp_v[g][HW + j - 1, rh, :] = hp
                    else:
                        sp_v[g][HW + Q - 1 + j, rh, :] = hp
                        sp_v[g][self.low + j, rh, :] = hp
                hraw_v[g][r, :] = piece(res, c, Q - 1)

        def fwd_u(self, g):
            lhs = []
            for c in range(NRC):
                r = pl.ds(g * RG + c * RC, RC)
                if self.first:
                    kk = jnp.concatenate([jnp.zeros((RC // 2, BK), u32), pltpu.bitcast(k_v[r, BK:], u32)], axis=1)
                else:
                    kk = pltpu.bitcast(k_v[r, :], u32)
                ks = None
                for tau in range(4):
                    shifted = kk if tau == 0 else pltpu.roll(kk, tau, 1)
                    term = _unpack(shifted[:, BK:]).astype(f32) * jnp.tile(col_v[tau, r, :], (1, Q))
                    ks = term if ks is None else ks + term
                kv = ks * v_v[r, :].astype(f32)
                for j in range(Q):
                    b = pltpu.bitcast(kv[:, _tile(j)].astype(bf16), u32)
                    kv_v[pl.ds((g * RG + c * RC) // 2, RC // 2), _tile(j)] = b
                    lhs.append(b)
            res = _dot(_unpack(jnp.concatenate(lhs, axis=0)), _unpack(ft_v[...]))
            for c in range(NRC):
                for j in range(Q):
                    sp_v[g][self.ub + j, pl.ds(c * RC, RC), :] = piece(res, c, j)

        def loader(self, g, p):
            seen = {}

            def load(blk):
                if blk not in seen:
                    seen[blk] = _halves(sp_v[g][blk, pl.ds(p * 8 + (HOFF if blk >= HL else 0), 8), :])
                return seen[blk]
            return load

        def link(self, z):
            return z if self.first else tuple(lax.select(self.keep, a, b) for a, b in zip(z, self.prev))

        def chain(self, load, init, terms):
            ar, ai = (None, None) if init is None else self.link(init)
            for j, m in terms:
                (ur, ui), (hr, hi) = load(j), load(m)
                if ar is None:
                    ar, ai = self.link((ur * hr, ur * hi))
                    ar, ai = ar - ui * hi, ai + ui * hr
                elif self.first:
                    ar, ai = ar + (ur * hr - ui * hi), ai + (ur * hi + ui * hr)
                else:
                    ar, ai = (ar + ur * hr) - ui * hi, (ai + ur * hi) + ui * hr
            self.prev = (ar, ai)
            return jnp.concatenate(self.prev, axis=1)

        def mac(self, p0, p1):
            for pp in range(p0, p1):
                g, p = divmod(pp, PG)
                pr = pl.ds(p * 8, 8)
                for a in range(Q):
                    if a % 2 == 0:
                        load = self.loader(g, p)
                    terms = [(self.ub + b, HL + a - b) for b in range(a + 1)]
                    init = None
                    if not self.first:
                        init = _halves(part_v[g][a, pr, :])
                        terms = [(U0 + b, HW + Q - 1 + a - b) for b in range(Q)] + terms
                    yf_v[g][a, pr, :] = self.chain(load, init, terms)

        def mac_ahead(self, p0, p1):
            for pp in range(p0, p1):
                g, p = divmod(pp, PG)
                pr, ph = pl.ds(p * 8, 8), pl.ds(p * 8 + HOFF, 8)
                for a in range(Q):
                    if a % 2 == 0:
                        load = self.loader(g, p)
                    terms = ([(UP + b, HW + Q - 1 + a - b) for b in range(Q)]
                             + [(UC + b, HL + Q + a - b) for b in range(Q)])
                    part_v[g][a, pr, :] = self.chain(load, None, terms)
                moves = [(UP + b, UC + b, pr) for b in range(Q)] + [(HW + b, HW + Q + b, ph) for b in range(Q - 1)]
                for dst, src, rows in moves:
                    sp_v[g][dst, rows, :] = jnp.concatenate(self.link(load(src)), axis=1)

    def inv_tile(t):
        lhs = [jnp.concatenate([yf_v[g][t], yf_v[g + 1][t]], axis=0).astype(bf16) for g in (0, 2)]
        conv = jnp.concatenate([_dot(a, _unpack(gt_v[...])) for a in lhs], axis=0)
        return conv + _unpack(kv_v[:, _tile(t)]).astype(f32) * col_v[4]

    def inv_group(g):
        rows = slice(g * RG, (g + 1) * RG)
        res = _dot(jnp.concatenate([yf_v[g][j] for j in range(Q)], axis=0).astype(bf16), _unpack(gt_v[...]))
        kv = _unpack(kv_v[g * RG // 2:(g + 1) * RG // 2, :]).astype(f32)
        for j in range(Q):
            y_v[rows, _tile(j)] = res[j * RG:(j + 1) * RG] + kv[:, _tile(j)] * col_v[4, rows, :]

    def stage(x, y):
        x = x + _ln(x) * y
        return x, _ln(x).astype(bf16)

    def mm1(xn):
        return _silu(_dot(_unpack(w1p_v[...]), xn))

    def head2(w, g0):
        return jnp.concatenate([_dot(w[:D // 2], g0), _dot(w[D // 2:], g0)], axis=0)

    def mm2(x, g):
        w, k0 = _unpack(w2p_v[...]), 2 * BK
        return x + (head2(w[:, :k0], g[:k0].astype(bf16)) + _dot(w[:, k0:], g[k0:].astype(bf16)))

    cv = Conv(0)
    for c in c_taps: c.wait()
    sh = sh_v[...].astype(f32)
    dd = d_v[...].astype(f32).reshape(1, D)
    for t in range(5):
        col_v[t] = jnp.broadcast_to(sh[t:t + 1, :] if t < 4 else dd, (BK, D)).T
    for c in c_h0: c.wait()
    for c in c_kv1 + [c_q0]: c.start()
    for g in range(NG): cv.fwd_h(g)
    for c in c_kv0: c.wait()
    for c in range(3): w1_copy(c).start()
    cv.fwd_u(0); cv.fwd_u(1)
    c_kv1[0].wait()
    cv.mac(0, 2 * PG)
    inv_group(0); inv_group(1)
    c_kv1[1].wait()
    w1_copy(3).start()
    cv.fwd_u(2); cv.fwd_u(3)

    def transpose_w1(c):
        w1p_v[W1B[c] // 2:W1B[c + 1] // 2, :] = pltpu.bitcast(w1_v[:, W1B[c]:W1B[c + 1]].T, u32)

    xs, xns, gs = [None] * Q, [None] * Q, [[] for _ in range(Q)]

    def mm1_part(c, t):
        g = _silu(_dot(_unpack(w1p_v[W1B[c] // 2:W1B[c + 1] // 2, :]), xns[t]))
        gs[t].append(g.astype(bf16))
        return g

    c_q0.wait()
    w1_copy(0).wait()
    c_w2.start()
    cv.mac(2 * PG, NP)
    inv_group(2); inv_group(3)
    transpose_w1(0)
    xs[0], xns[0] = stage(q_v[:, _tile(0)].astype(f32), y_v[:, _tile(0)])
    w1_copy(1).wait(); w1_copy(2).wait()
    transpose_w1(1); transpose_w1(2)
    keep = all_true()
    for t in range(Q):
        for c in range(3 if t < Q - 1 else 2):
            g = mm1_part(c, t)
            if c == 0 and t + 1 < Q:
                x = tie(q_v[:, _tile(t + 1)].astype(f32), keep, g[0:8])
                xs[t + 1], xns[t + 1] = stage(x, y_v[:, _tile(t + 1)])
    w1_copy(3).wait()
    transpose_w1(3)
    keep = all_true()
    mm1_part(2, Q - 1)
    paced = []
    for t in range(Q - 1):
        g = mm1_part(3, t)
        paced += [g[i * 8:(i + 1) * 8] for i in range(0, 96, 9)]
    for i in range(2 * NG * Q):
        z = jnp.tile(jnp.where(keep, 0.0, paced[i]), (PG, 2))
        g, a = divmod(i % (NG * Q), Q)
        if i < NG * Q:
            part_v[g][a] = z
        else:
            sp_v[g][UP + a, :RG] = z
    c_w2.wait()
    for c in conv_copies(1): c.start()
    mm1_part(3, Q - 1)
    for c in range(W1C):
        gc_v[W1B[c] // 2:W1B[c + 1] // 2, :] = pltpu.bitcast(gs[Q - 1][c], u32)
    x1_v[...] = xs[Q - 1]
    w2t = w2t_v[...]
    w2p_v[...] = pltpu.bitcast(w2t, u32)
    for t in range(Q - 1):
        acc = head2(w2t[:, :W1B[1]], gs[t][0])
        for c in range(1, W1C):
            acc = acc + _dot(w2t[:, W1B[c]:W1B[c + 1]], gs[t][c])
        x2_v[:, _tile(t)] = xs[t] + acc

    def step(s, carry):
        for c in conv_copies(s + 1): c.wait()
        c_q = step_copy(q_hbm, q_v, s + 1, sem.at[4])
        c_q.start()
        cv = Conv(s + 1)
        o0 = pl.multiple_of(s * T, T)

        w2, gc = _unpack(w2p_v[...]), _unpack(gc_v[...])
        part = lambda a, b: (w2[:, a * BK:b * BK], gc[a * BK:b * BK])
        cv.fwd_h(0); acc = x1_v[...] + _dot(*part(0, 2))
        cv.fwd_u(0); cv.fwd_h(1)
        cv.fwd_u(1); cv.fwd_h(2)
        cv.fwd_u(2); cv.fwd_h(3)
        cv.fwd_u(3); acc = acc + _dot(*part(2, 4))
        hd = head2(*part(4, 6))
        x2_v[:, _tile(Q - 1)] = acc + hd + _dot(*part(6, F // BK))
        x, xn = stage(x2_v[:, _tile(0)], tie(y_v[:, _tile(0)], cv.keep, hd[D - 8:]))
        c_q.wait()

        @pl.when(s + 2 < NS)
        def _():
            for c in conv_copies(s + 2): c.start()

        for t in range(Q):
            g = mm1(xn)
            cv.anchor(g[0:8])
            if t < Q - 1:
                cv.mac(CB[t], CB[t + 1])
            cv.mac_ahead(BB[t], BB[t + 1])
            if t == Q - 1:
                y = inv_tile(0)
            o_v[:, pl.ds(o0 + t * BK, BK)] = mm2(x, g).astype(bf16)
            if t < Q - 1:
                x, xn = stage(x2_v[:, _tile(t + 1)], y_v[:, _tile(t + 1)])
        for t in range(Q):
            x, xn = stage(q_v[:, _tile(t)].astype(f32), y)
            y_v[:, _tile(t)] = y
            g = mm1(xn)
            if t + 1 < Q:
                cv.anchor(g[0:8])
                cv.mac_ahead(BB[Q + t], BB[Q + t + 1])
                y = inv_tile(t + 1)
                x2_v[:, _tile(t)] = mm2(x, g)
            else:
                gc_v[...] = pltpu.bitcast(g.astype(bf16), u32)
                x1_v[...] = x
        out_copy(o0, T).start()
        return carry

    lax.fori_loop(0, NS - 1, step, 0)

    x2_v[:, _tile(Q - 1)] = mm2(x1_v[...], _unpack(gc_v[...]))
    for t in range(Q):
        x, xn = stage(x2_v[:, _tile(t)], y_v[:, _tile(t)])
        c0 = (NS - 1) * T + t * BK
        if t < Q - 1:
            o_v[:, c0:c0 + BK] = mm2(x, mm1(xn)).astype(bf16)
            out_copy(c0, BK).start()
        else:
            g, w = mm1(xn).astype(bf16), _unpack(w2p_v[...])
            for r0, r1 in LAST:
                o_v[r0:r1, c0:] = (x[r0:r1] + _dot(w[r0:r1], g)).astype(bf16)
                at = (pl.ds(r0, r1 - r0), pl.ds(c0, BK))
                pltpu.make_async_copy(o_v.at[at], o_hbm.at[at], osem).start()
    out_copy(0, S).wait()


def _compiler_params():
    base = dict(vmem_limit_bytes=64 * 1024 * 1024, disable_bounds_checks=True)
    try:
        return pltpu.CompilerParams(disable_semaphore_checks=True, **base)
    except TypeError:
        return pltpu.CompilerParams(**base)


@jax.jit
def pallas_interleave_layers__ssm_conv_h3__dense_activation_silu__prompt_kernel(
        A_q, A_k, A_v, A_shift_k, A_ssm_k, A_ssm_D, B_x, B_w1, B_w2):
    act = pltpu.VMEM((D, T), bf16)
    wgt = pltpu.VMEM((D, F), bf16)
    groups = ([pltpu.VMEM((NSP, RG + 2 * HOFF, 2 * BK), f32)] * NG + [pltpu.VMEM((RG, 2 * BK), f32)] * NG
              + [pltpu.VMEM((Q, RG, 2 * BK), f32)] * (2 * NG))
    out = pl.pallas_call(
        _kernel,
        in_specs=[pl.BlockSpec(memory_space=pl.ANY)] * 8,
        out_specs=pl.BlockSpec(memory_space=pl.ANY),
        out_shape=jax.ShapeDtypeStruct((D, S), bf16),
        scratch_shapes=[act, pltpu.VMEM((D, T + BK), bf16), act, act, pltpu.VMEM((D, S), bf16)] + [
            pltpu.VMEM((4, D), bf16), pltpu.VMEM((D,), bf16), wgt, wgt,
            pltpu.VMEM((F // 2, D), u32), pltpu.VMEM((D // 2, F), u32),
            pltpu.VMEM((BK // 2, 2 * BK), u32), pltpu.VMEM((BK, BK), u32),
            pltpu.VMEM((5, D, BK), f32), pltpu.VMEM((8, BK), i32),
            pltpu.VMEM((D // 2, T), u32), pltpu.VMEM((D, T), f32), pltpu.VMEM((D, T), f32),
            pltpu.VMEM((F // 2, BK), u32), pltpu.VMEM((D, BK), f32),
            pltpu.SemaphoreType.DMA((8,)), pltpu.SemaphoreType.DMA((W1C,)), pltpu.SemaphoreType.DMA] + groups,
        compiler_params=_compiler_params(),
    )(A_q.reshape(S, D).T, A_k.reshape(S, D).T, A_v.reshape(S, D).T, A_shift_k.T, A_ssm_k, A_ssm_D,
      B_w1, B_w2.T)
    return out.T.reshape(1, S, D)
```

```python
import jax
import jax.numpy as jnp
import numpy as np
from jax import lax
import jax.experimental.pallas as pl
import jax.experimental.pallas.tpu as pltpu

S, D, F = 2048, 448, 1792
BK = 128
T = 512
Q = T // BK
NS = S // T
RG = 112
NG = D // RG
PG = RG // 8
NP = NG * PG
RC = 16
NRC = RG // RC
W1B = (0, 256, 512, 1024, 1792)
W1C = len(W1B) - 1
U0, UC, UP, HL, HW, NSP = 0, 4, 8, 12, 24, 31
HOFF = 8
CB = (0, 19, 38, 56)
BB = (0, 2, 5, 9, 20, 32, 44, 56)
EPS = 1e-5
LAST = ((0, 208), (208, 416), (416, 448))
f32, bf16, u32, i32 = jnp.float32, jnp.bfloat16, jnp.uint32, jnp.int32


def _dft_table(shape, n_axis, scale):
    n = lax.broadcasted_iota(i32, shape, n_axis)
    kk = lax.broadcasted_iota(i32, shape, 1 - n_axis)
    ph = (4 * (kk & (BK - 1)) + 1) * n - (kk & BK)
    phi = ((ph & (2 * BK - 1)) - BK).astype(f32) * (np.pi / (2 * BK))
    p2 = phi * phi
    s = 1.0 / 39916800
    for d in (362880, 5040, 120, 6, 1):
        s = 1.0 / d - p2 * s
    s = s * phi
    return (jnp.where((ph & (2 * BK)) == 0, -scale, scale) * s).astype(bf16)


def _ln(x):
    m = jnp.sum(x, axis=0, keepdims=True) * (1.0 / D)
    xc = x - m
    v = jnp.sum(xc * xc, axis=0, keepdims=True) * (1.0 / D)
    return xc * lax.rsqrt(v + EPS)


def _silu(h):
    t = 0.5 * h
    return t * jnp.tanh(t) + t


def _dot(a, b):
    return jnp.dot(a, b, preferred_element_type=f32)


def _unpack(x):
    return pltpu.bitcast(x, bf16)


def _halves(z):
    return z[:, :BK], z[:, BK:]


def _tile(t):
    return slice(t * BK, (t + 1) * BK)


def _kernel(q_hbm, k_hbm, v_hbm, sh_hbm, h_hbm, d_hbm, w1_hbm, w2t_hbm, o_hbm,
            q_v, k_v, v_v, h_v, o_v, sh_v, d_v, w1_v, w2t_v, w1p_v, w2p_v, ft_v, gt_v, col_v, zero_v,
            kv_v, y_v, x2_v, gc_v, x1_v, sem, wsem, osem, *grp):
    sp_v, hraw_v, part_v, yf_v = (grp[i * NG:(i + 1) * NG] for i in range(4))

    def step_copy(src, dst, s, sm, halo=0):
        return pltpu.make_async_copy(src.at[:, pl.ds(pl.multiple_of(s * T - halo, BK), T + halo)], dst, sm)

    def conv_copies(s):
        return [step_copy(k_hbm, k_v, s, sem.at[6], BK), step_copy(v_hbm, v_v, s, sem.at[6]),
                step_copy(h_hbm, h_v, s, sem.at[6])]

    def half_copies(hh, sk, sv):
        rows = pl.ds(hh * 2 * RG, 2 * RG)
        return [pltpu.make_async_copy(k_hbm.at[rows, pl.ds(0, T)], k_v.at[rows, pl.ds(BK, T)], sk),
                pltpu.make_async_copy(v_hbm.at[rows, pl.ds(0, T)], v_v.at[rows], sv)]

    def w1_copy(c):
        cols = pl.ds(W1B[c], W1B[c + 1] - W1B[c])
        return pltpu.make_async_copy(w1_hbm.at[:, cols], w1_v.at[:, cols], wsem.at[c])

    def out_copy(c0, w):
        cols = pl.ds(c0, w)
        return pltpu.make_async_copy(o_v.at[:, cols], o_hbm.at[:, cols], osem)

    c_taps = [pltpu.make_async_copy(sh_hbm, sh_v, sem.at[0]), pltpu.make_async_copy(d_hbm, d_v, sem.at[0])]
    c_h0 = [step_copy(h_hbm, h_v, 0, sem.at[1])]
    c_kv0 = half_copies(0, sem.at[2], sem.at[2])
    c_kv1 = half_copies(1, sem.at[7], sem.at[3])
    c_q0, c_q1 = (pltpu.make_async_copy(q_hbm.at[:, pl.ds(i * T // 2, T // 2)], q_v.at[:, pl.ds(i * T // 2, T // 2)],
                                        sem.at[4 * i + 4]) for i in range(2))
    c_w2 = pltpu.make_async_copy(w2t_hbm, w2t_v, sem.at[5])
    for c in c_taps + c_h0 + c_kv0:
        c.start()
    zero_v[...] = jnp.zeros(zero_v.shape, i32)
    ft_v[...] = pltpu.bitcast(_dft_table((BK, 2 * BK), 0, 1.0), u32)
    gt_v[...] = pltpu.bitcast(_dft_table((2 * BK, BK), 1, 1.0 / BK), u32)

    def all_true():
        return zero_v[...] == 0

    def tie(val, keep, dep):
        return jnp.concatenate([lax.select(keep, val[0:8], dep), val[8:]], axis=0)

    def piece(res, c, j):
        return res[(c * Q + j) * RC:(c * Q + j + 1) * RC]

    class Conv:
        def __init__(self, q):
            self.q = q
            self.first = isinstance(q, int)
            self.ub = U0 if self.first else UC
            self.keep = None if self.first else all_true()
            self.low = None if self.first else HL + Q * jnp.minimum(q, 2)
            self.prev = None
            self.paced = not self.first

        def anchor(self, val):
            self.prev = (val, val)

        def fwd_h(self, g):
            hh = h_v[pl.ds(g * RG, RG), :]
            lhs = jnp.concatenate([hh[c * RC:(c + 1) * RC, _tile(j)] for c in range(NRC) for j in range(Q)], axis=0)
            res = _dot(lhs, _unpack(ft_v[...]))
            for c in range(NRC):
                r = pl.ds(c * RC, RC)
                rh = pl.ds(c * RC + HOFF, RC)
                for j in range(Q):
                    hp = piece(res, c, j)
                    if j > 0 or not self.first:
                        prev = hraw_v[g][r, :] if j == 0 else piece(res, c, j - 1)
                        hp = jnp.concatenate([hp[:, :BK] + prev[:, BK:], hp[:, BK:] - prev[:, :BK]], axis=1)
                    if self.first:
                        sp_v[g][HL + j, rh, :] = hp
                        if j > 0:
                            sp_v[g][HW + j - 1, rh, :] = hp
                    else:
                        sp_v[g][HW + Q - 1 + j, rh, :] = hp
                        sp_v[g][self.low + j, rh, :] = hp
                hraw_v[g][r, :] = piece(res, c, Q - 1)

        def fwd_u(self, g):
            lhs = []
            for c in range(NRC):
                r = pl.ds(g * RG + c * RC, RC)
                if self.first:
                    kk = jnp.concatenate([jnp.zeros((RC // 2, BK), u32), pltpu.bitcast(k_v[r, BK:], u32)], axis=1)
                else:
                    kk = pltpu.bitcast(k_v[r, :], u32)
                ks = None
                for tau in range(4):
                    shifted = kk if tau == 0 else pltpu.roll(kk, tau, 1)
                    term = _unpack(shifted[:, BK:]).astype(f32) * jnp.tile(col_v[tau, r, :], (1, Q))
                    ks = term if ks is None else ks + term
                kv = ks * v_v[r, :].astype(f32)
                for j in range(Q):
                    b = pltpu.bitcast(kv[:, _tile(j)].astype(bf16), u32)
                    kv_v[pl.ds((g * RG + c * RC) // 2, RC // 2), _tile(j)] = b
                    lhs.append(b)
            res = _dot(_unpack(jnp.concatenate(lhs, axis=0)), _unpack(ft_v[...]))
            for c in range(NRC):
                for j in range(Q):
                    sp_v[g][self.ub + j, pl.ds(c * RC, RC), :] = piece(res, c, j)

        def loader(self, g, p):
            seen = {}

            def load(blk):
                if blk not in seen:
                    seen[blk] = _halves(sp_v[g][blk, pl.ds(p * 8 + (HOFF if blk >= HL else 0), 8), :])
                return seen[blk]
            return load

        def link(self, z):
            return z if not self.paced else tuple(lax.select(self.keep, a, b) for a, b in zip(z, self.prev))

        def chain(self, load, init, terms):
            ar, ai = (None, None) if init is None else self.link(init)
            for j, m in terms:
                (ur, ui), (hr, hi) = load(j), load(m)
                if ar is None:
                    ar, ai = self.link((ur * hr, ur * hi))
                    ar, ai = ar - ui * hi, ai + ui * hr
                elif not self.paced:
                    ar, ai = ar + (ur * hr - ui * hi), ai + (ur * hi + ui * hr)
                else:
                    ar, ai = (ar + ur * hr) - ui * hi, (ai + ur * hi) + ui * hr
            self.prev = (ar, ai)
            return jnp.concatenate(self.prev, axis=1)

        def mac(self, p0, p1, outs=range(Q)):
            for pp in range(p0, p1):
                g, p = divmod(pp, PG)
                pr = pl.ds(p * 8, 8)
                for a in outs:
                    if a % 2 == 0:
                        load = self.loader(g, p)
                    terms = [(self.ub + b, HL + a - b) for b in range(a + 1)]
                    init = None
                    if not self.first:
                        init = _halves(part_v[g][a, pr, :])
                        terms = [(U0 + b, HW + Q - 1 + a - b) for b in range(Q)] + terms
                    yf_v[g][a, pr, :] = self.chain(load, init, terms)

        def mac_ahead(self, p0, p1):
            for pp in range(p0, p1):
                g, p = divmod(pp, PG)
                pr, ph = pl.ds(p * 8, 8), pl.ds(p * 8 + HOFF, 8)
                for a in range(Q):
                    if a % 2 == 0:
                        load = self.loader(g, p)
                    terms = ([(UP + b, HW + Q - 1 + a - b) for b in range(Q)]
                             + [(UC + b, HL + Q + a - b) for b in range(Q)])
                    part_v[g][a, pr, :] = self.chain(load, None, terms)
                moves = [(UP + b, UC + b, pr) for b in range(Q)] + [(HW + b, HW + Q + b, ph) for b in range(Q - 1)]
                for dst, src, rows in moves:
                    sp_v[g][dst, rows, :] = jnp.concatenate(self.link(load(src)), axis=1)

    def inv_tile(t):
        lhs = [jnp.concatenate([yf_v[g][t], yf_v[g + 1][t]], axis=0).astype(bf16) for g in (0, 2)]
        conv = jnp.concatenate([_dot(a, _unpack(gt_v[...])) for a in lhs], axis=0)
        return conv + _unpack(kv_v[:, _tile(t)]).astype(f32) * col_v[4]

    def inv_group(g):
        rows = slice(g * RG, (g + 1) * RG)
        res = _dot(jnp.concatenate([yf_v[g][j] for j in range(Q)], axis=0).astype(bf16), _unpack(gt_v[...]))
        kv = _unpack(kv_v[g * RG // 2:(g + 1) * RG // 2, :]).astype(f32)
        for j in range(Q):
            y_v[rows, _tile(j)] = res[j * RG:(j + 1) * RG] + kv[:, _tile(j)] * col_v[4, rows, :]

    def inv_low(t):
        rows = slice(2 * RG, D)
        res = _dot(jnp.concatenate([yf_v[2][t], yf_v[3][t]], axis=0).astype(bf16), _unpack(gt_v[...]))
        y_v[rows, _tile(t)] = res + _unpack(kv_v[RG:, _tile(t)]).astype(f32) * col_v[4, rows, :]

    def stage(x, y):
        x = x + _ln(x) * y
        return x, _ln(x).astype(bf16)

    def mm1(xn):
        return _silu(_dot(_unpack(w1p_v[...]), xn))

    def head2(w, g0):
        return jnp.concatenate([_dot(w[:D // 2], g0), _dot(w[D // 2:], g0)], axis=0)

    def mm2(x, g):
        w, k0 = _unpack(w2p_v[...]), 2 * BK
        return x + (head2(w[:, :k0], g[:k0].astype(bf16)) + _dot(w[:, k0:], g[k0:].astype(bf16)))

    cv = Conv(0)
    for c in c_taps: c.wait()
    sh = sh_v[...].astype(f32)
    dd = d_v[...].astype(f32).reshape(1, D)
    for t in range(5):
        col_v[t] = jnp.broadcast_to(sh[t:t + 1, :] if t < 4 else dd, (BK, D)).T
    for c in c_h0: c.wait()
    for c in c_kv1 + [c_q0]: c.start()
    for g in range(NG): cv.fwd_h(g)
    for c in c_kv0: c.wait()
    for c in range(3): w1_copy(c).start()
    cv.fwd_u(0); cv.fwd_u(1)
    c_kv1[0].wait()
    cv.mac(0, 2 * PG)
    inv_group(0); inv_group(1)
    c_kv1[1].wait()
    c_q1.start(); w1_copy(3).start()
    cv.fwd_u(2); cv.fwd_u(3)

    def transpose_w1(c):
        w1p_v[W1B[c] // 2:W1B[c + 1] // 2, :] = pltpu.bitcast(w1_v[:, W1B[c]:W1B[c + 1]].T, u32)

    xs, xns, gs = [None] * Q, [None] * Q, [[] for _ in range(Q)]

    def mm1_part(c, t):
        g = _silu(_dot(_unpack(w1p_v[W1B[c] // 2:W1B[c + 1] // 2, :]), xns[t]))
        gs[t].append(g.astype(bf16))
        return g

    c_q0.wait()
    w1_copy(0).wait()
    c_w2.start()
    cv.mac(2 * PG, NP, (0, 1))
    inv_low(0); inv_low(1)
    transpose_w1(0)
    for t in range(2):
        xs[t], xns[t] = stage(q_v[:, _tile(t)].astype(f32), y_v[:, _tile(t)])
    w1_copy(1).wait(); w1_copy(2).wait()
    transpose_w1(1); transpose_w1(2)
    cv.keep, cv.paced = all_true(), True
    cv.anchor(mm1_part(0, 0)[0:8])
    cv.mac(2 * PG, NP, (2, 3))
    mm1_part(1, 0); mm1_part(2, 0); mm1_part(0, 1)
    inv_low(2); inv_low(3)
    mm1_part(1, 1)
    w1_copy(3).wait(); c_q1.wait()
    transpose_w1(3)
    for t in range(2, Q):
        xs[t], xns[t] = stage(q_v[:, _tile(t)].astype(f32), y_v[:, _tile(t)])
    mm1_part(2, 1); mm1_part(3, 0); mm1_part(3, 1)
    late = [mm1_part(c, 2) for c in range(W1C)][:-1] + [mm1_part(c, 3) for c in range(W1C - 1)]
    late = jnp.concatenate(late, axis=0)
    paced = [late[i * 64:i * 64 + 8] for i in range(2 * NG * Q)]
    keep = all_true()
    for i in range(2 * NG * Q):
        z = jnp.tile(jnp.where(keep, 0.0, paced[i]), (PG, 2))
        g, a = divmod(i % (NG * Q), Q)
        if i < NG * Q:
            part_v[g][a] = z
        else:
            sp_v[g][UP + a, :RG] = z
    c_w2.wait()
    for c in conv_copies(1): c.start()
    mm1_part(3, Q - 1)
    for c in range(W1C):
        gc_v[W1B[c] // 2:W1B[c + 1] // 2, :] = pltpu.bitcast(gs[Q - 1][c], u32)
    x1_v[...] = xs[Q - 1]
    w2t = w2t_v[...]
    w2p_v[...] = pltpu.bitcast(w2t, u32)
    for t in range(Q - 1):
        acc = head2(w2t[:, :W1B[1]], gs[t][0])
        for c in range(1, W1C):
            acc = acc + _dot(w2t[:, W1B[c]:W1B[c + 1]], gs[t][c])
        x2_v[:, _tile(t)] = xs[t] + acc

    def step(s, carry):
        for c in conv_copies(s + 1): c.wait()
        c_q = step_copy(q_hbm, q_v, s + 1, sem.at[4])
        c_q.start()
        cv = Conv(s + 1)
        o0 = pl.multiple_of(s * T, T)

        w2, gc = _unpack(w2p_v[...]), _unpack(gc_v[...])
        part = lambda a, b: (w2[:, a * BK:b * BK], gc[a * BK:b * BK])
        cv.fwd_h(0); acc = x1_v[...] + _dot(*part(0, 2))
        cv.fwd_u(0); cv.fwd_h(1)
        cv.fwd_u(1); cv.fwd_h(2)
        cv.fwd_u(2); cv.fwd_h(3)
        cv.fwd_u(3); acc = acc + _dot(*part(2, 4))
        hd = head2(*part(4, 6))
        x2_v[:, _tile(Q - 1)] = acc + hd + _dot(*part(6, F // BK))
        x, xn = stage(x2_v[:, _tile(0)], tie(y_v[:, _tile(0)], cv.keep, hd[D - 8:]))
        c_q.wait()

        @pl.when(s + 2 < NS)
        def _():
            for c in conv_copies(s + 2): c.start()

        for t in range(Q):
            g = mm1(xn)
            cv.anchor(g[0:8])
            if t < Q - 1:
                cv.mac(CB[t], CB[t + 1])
            cv.mac_ahead(BB[t], BB[t + 1])
            if t == Q - 1:
                y = inv_tile(0)
            o_v[:, pl.ds(o0 + t * BK, BK)] = mm2(x, g).astype(bf16)
            if t < Q - 1:
                x, xn = stage(x2_v[:, _tile(t + 1)], y_v[:, _tile(t + 1)])
        for t in range(Q):
            x, xn = stage(q_v[:, _tile(t)].astype(f32), y)
            y_v[:, _tile(t)] = y
            g = mm1(xn)
            if t + 1 < Q:
                cv.anchor(g[0:8])
                cv.mac_ahead(BB[Q + t], BB[Q + t + 1])
                y = inv_tile(t + 1)
                x2_v[:, _tile(t)] = mm2(x, g)
            else:
                gc_v[...] = pltpu.bitcast(g.astype(bf16), u32)
                x1_v[...] = x
        out_copy(o0, T).start()
        return carry

    lax.fori_loop(0, NS - 1, step, 0)

    x2_v[:, _tile(Q - 1)] = mm2(x1_v[...], _unpack(gc_v[...]))
    for t in range(Q):
        x, xn = stage(x2_v[:, _tile(t)], y_v[:, _tile(t)])
        c0 = (NS - 1) * T + t * BK
        if t < Q - 1:
            o_v[:, c0:c0 + BK] = mm2(x, mm1(xn)).astype(bf16)
            out_copy(c0, BK).start()
        else:
            g, w = mm1(xn).astype(bf16), _unpack(w2p_v[...])
            for r0, r1 in LAST:
                o_v[r0:r1, c0:] = (x[r0:r1] + _dot(w[r0:r1], g)).astype(bf16)
                at = (pl.ds(r0, r1 - r0), pl.ds(c0, BK))
                pltpu.make_async_copy(o_v.at[at], o_hbm.at[at], osem).start()
    out_copy(0, S).wait()


def _compiler_params():
    base = dict(vmem_limit_bytes=64 * 1024 * 1024, disable_bounds_checks=True)
    try:
        return pltpu.CompilerParams(disable_semaphore_checks=True, **base)
    except TypeError:
        return pltpu.CompilerParams(**base)


@jax.jit
def pallas_interleave_layers__ssm_conv_h3__dense_activation_silu__prompt_kernel(
        A_q, A_k, A_v, A_shift_k, A_ssm_k, A_ssm_D, B_x, B_w1, B_w2):
    act = pltpu.VMEM((D, T), bf16)
    wgt = pltpu.VMEM((D, F), bf16)
    groups = ([pltpu.VMEM((NSP, RG + 2 * HOFF, 2 * BK), f32)] * NG + [pltpu.VMEM((RG, 2 * BK), f32)] * NG
              + [pltpu.VMEM((Q, RG, 2 * BK), f32)] * (2 * NG))
    out = pl.pallas_call(
        _kernel,
        in_specs=[pl.BlockSpec(memory_space=pl.ANY)] * 8,
        out_specs=pl.BlockSpec(memory_space=pl.ANY),
        out_shape=jax.ShapeDtypeStruct((D, S), bf16),
        scratch_shapes=[act, pltpu.VMEM((D, T + BK), bf16), act, act, pltpu.VMEM((D, S), bf16)] + [
            pltpu.VMEM((4, D), bf16), pltpu.VMEM((D,), bf16), wgt, wgt,
            pltpu.VMEM((F // 2, D), u32), pltpu.VMEM((D // 2, F), u32),
            pltpu.VMEM((BK // 2, 2 * BK), u32), pltpu.VMEM((BK, BK), u32),
            pltpu.VMEM((5, D, BK), f32), pltpu.VMEM((8, BK), i32),
            pltpu.VMEM((D // 2, T), u32), pltpu.VMEM((D, T), f32), pltpu.VMEM((D, T), f32),
            pltpu.VMEM((F // 2, BK), u32), pltpu.VMEM((D, BK), f32),
            pltpu.SemaphoreType.DMA((9,)), pltpu.SemaphoreType.DMA((W1C,)), pltpu.SemaphoreType.DMA] + groups,
        compiler_params=_compiler_params(),
    )(A_q.reshape(S, D).T, A_k.reshape(S, D).T, A_v.reshape(S, D).T, A_shift_k.T, A_ssm_k, A_ssm_D,
      B_w1, B_w2.T)
    return out.T.reshape(1, S, D)
```
